```python
import os as _os
_os.environ.setdefault("JAX_PLATFORMS", "cpu")
import jax
import jax.numpy as jnp

def _softmax(x, axis=-1):
    return jax.nn.softmax(x, axis=axis)
def _gelu(x):
    return jax.nn.gelu(x, approximate=True)
def _silu(x):
    return jax.nn.silu(x)
def _sigmoid(x):
    return jax.nn.sigmoid(x)
def _layernorm(x, axis=-1, eps=1e-5):
    m = jnp.mean(x, axis=axis, keepdims=True)
    v = jnp.var(x, axis=axis, keepdims=True)
    return (x - m) / jnp.sqrt(v + eps)
def _scatter_add(tgt, idx, src, axis=0):
    return tgt.at[idx].add(src)
def _segment_sum(src, seg, n):
    return jax.ops.segment_sum(src, seg, n)
class _Rng:
    def __init__(self, key):
        self._k = key
    def _next(self):
        self._k, sub = jax.random.split(self._k)
        return sub
    def normal(self, shape):
        return jax.random.normal(self._next(), shape, dtype=jnp.bfloat16)
    def randint(self, lo, hi, shape):
        return jax.random.randint(self._next(), shape, lo, hi, dtype=jnp.int32)
    def uniform(self, shape, lo=0.0, hi=1.0):
        return jax.random.uniform(self._next(), shape, jnp.bfloat16, lo, hi)
    def permutation(self, n):
        return jax.random.permutation(self._next(), n)


kernel_name = 'parallel_sum__softmax_full_mha__glu_gated_swiglu__prompt'

def setup_inputs():
    _rng = _Rng(jax.random.key(int.from_bytes(__import__("os").urandom(4), "little")))
    _w = (lambda a: (lambda t: t.astype(jnp.bfloat16) if jnp.issubdtype(t.dtype, jnp.floating) else t)(jnp.asarray(a)))
    def _A_setup():
        B, S, D = 1, 2048, 448
        return {
            "x": _w((lambda *s: _rng.normal(s) * 0.05)(B, S, D)),
            "wqkv": _w((lambda *s: _rng.normal(s) * 0.05)(D, 3 * D)),
            "wo": _w((lambda *s: _rng.normal(s) * 0.05)(D, D)),
        }
    _A_in = _A_setup()

    def _B_setup():
        B, S, D, F = 1, 2048, 448, 1792
        return {
            "x": _w((lambda *s: _rng.normal(s) * 0.05)(B, S, D)),
            "w1": _w((lambda *s: _rng.normal(s) * 0.05)(D, F) * (2.0 / D) ** 0.5),
            "w3": _w((lambda *s: _rng.normal(s) * 0.05)(D, F) * (2.0 / D) ** 0.5),
            "w2": _w((lambda *s: _rng.normal(s) * 0.05)(F, D) * (2.0 / F) ** 0.5),
        }
    _B_in = _B_setup()

    return {
        "A_x": _A_in["x"],
        "A_wqkv": _A_in["wqkv"],
        "A_wo": _A_in["wo"],
        "B_x": _B_in["x"],
        "B_w1": _B_in["w1"],
        "B_w3": _B_in["w3"],
        "B_w2": _B_in["w2"],
    }

def reference(A_x, A_wqkv, A_wo, B_x, B_w1, B_w3, B_w2):
    def _A_ref(x, wqkv, wo):
        B, S, D = x.shape
        H = 16; Dh = D // H
        qkv = (lambda x, *d: x.transpose(*d))((x @ wqkv).reshape(B, S, 3, H, Dh), 2, 0, 3, 1, 4)
        q, k, v = qkv[0], qkv[1], qkv[2]
        scale = Dh ** -0.5
        scores = jnp.einsum("bhqd,bhkd->bhqk", q, k) * scale
        p = _softmax(scores, axis=-1)
        o = jnp.einsum("bhqk,bhkd->bhqd", p, v)
        return (lambda x, *d: x.transpose(*d))(o, 0, 2, 1, 3).reshape(B, S, D) @ wo

    def _B_ref(x, w1, w3, w2):
        gate = jnp.einsum("bsd,df->bsf", x, w1)
        up = jnp.einsum("bsd,df->bsf", x, w3)
        h = _silu(gate) * up
        out = jnp.einsum("bsf,fd->bsd", h, w2)
        return out

    x = A_x
    xn = _layernorm(x, axis=-1)
    return x + _A_ref(xn, A_wqkv, A_wo) + _B_ref(xn, B_w1, B_w3, B_w2)
```

```python
import functools, math
import jax, jax.numpy as jnp
from jax import lax
from jax.experimental import pallas as pl
from jax.experimental.pallas import tpu as pltpu

S, D, H, DH, F = 2048, 448, 16, 28, 1792
NG, GW = 4, 112
EPS = 1e-5
QSCALE = (DH ** -0.5) * math.log2(math.e)
NT = (((1,), (1,)), ((), ()))
f32, bf16 = jnp.float32, jnp.bfloat16

def build(TQ=512, TA=512, KC=256, TF=512, FC=256, OPAQUE=True, DO_ATT=True, DO_FFN=True):
    NQ = S // TQ
    NC = S // KC

    def kernel(xt_hbm, wqkv_hbm, wo_hbm, w1_hbm, w3_hbm, w2t_hbm, out_hbm,
               xt_ref, wqkv_ref, wo_ref, w1_ref, w3_ref, w2t_ref, outb_ref,
               wt_ref, wqv_ref, wk_ref, wot_ref,
               xn_ref, qt_ref, k_ref, vt_ref, ot_ref, sa_ref, sb_ref, z_ref, sems, osems):
        cp_wqkv = pltpu.make_async_copy(wqkv_hbm, wqkv_ref, sems.at[0])
        cp_x = pltpu.make_async_copy(xt_hbm, xt_ref, sems.at[1])
        cp_wo = pltpu.make_async_copy(wo_hbm, wo_ref, sems.at[2])
        cp_w1 = pltpu.make_async_copy(w1_hbm, w1_ref, sems.at[3])
        cp_w3 = pltpu.make_async_copy(w3_hbm, w3_ref, sems.at[4])
        cp_w2 = pltpu.make_async_copy(w2t_hbm, w2t_ref, sems.at[5])
        for cp in (cp_wqkv, cp_x, cp_wo, cp_w1, cp_w3, cp_w2):
            cp.start()
        z_ref[0] = 0
        z_ref[1] = 0

        cp_wqkv.wait()
        wt_ref[...] = wqkv_ref[...].astype(f32).T
        wqv_ref[0:D, :] = wt_ref[0:D, :].astype(bf16)
        zpad4 = jnp.zeros((32 - DH, D), f32)
        for h in range(H):
            blk = jnp.concatenate([wt_ref[2 * D + h * DH: 2 * D + (h + 1) * DH, :], zpad4], axis=0)
            wqv_ref[D + 32 * h: D + 32 * (h + 1), :] = blk.astype(bf16)
        for g in range(NG):
            wk_ref[128 * g:128 * g + GW, :] = wt_ref[D + GW * g: D + GW * (g + 1), :].astype(bf16)
            wk_ref[128 * g + GW:128 * (g + 1), :] = jnp.zeros((128 - GW, D), bf16)

        cp_x.wait()
        for c in range(S // TA):
            sl = slice(c * TA, (c + 1) * TA)
            xt = xt_ref[:, sl].astype(f32)
            mu = jnp.sum(xt, axis=0, keepdims=True) * (1.0 / D)
            xc = xt - mu
            var = jnp.sum(xc * xc, axis=0, keepdims=True) * (1.0 / D)
            xnt = xc * lax.rsqrt(var + EPS)
            xn = xnt.T.astype(bf16)
            xn_ref[sl, :] = xn
            qv = jnp.dot(wqv_ref[...], xnt.astype(bf16), preferred_element_type=f32)
            for g in range(NG):
                qt_ref[g, 0:GW, sl] = (qv[GW * g:GW * (g + 1), :] * QSCALE).astype(bf16)
                qt_ref[g, GW:128, sl] = jnp.zeros((128 - GW, TA), bf16)
            row = lax.broadcasted_iota(jnp.int32, (32, TA), 0)
            for h in range(H):
                vt_ref[h, :, sl] = jnp.where(row == DH, 1.0, qv[D + 32 * h:D + 32 * (h + 1), :]).astype(bf16)
            kk = lax.dot_general(xn, wk_ref[...], NT, preferred_element_type=f32)
            for g in range(NG):
                k_ref[g, sl, :] = kk[:, 128 * g:128 * (g + 1)].astype(bf16)

        rowq = lax.broadcasted_iota(jnp.int32, (128, TQ), 0)

        def make_qm(g, j, q0):
            q = qt_ref[g, :, pl.ds(q0, TQ)]
            return jnp.where((rowq >= j * DH) & (rowq < (j + 1) * DH), q.astype(f32), 0.0).astype(bf16)

        def srows(c, which):
            if OPAQUE:
                return pl.ds(pl.multiple_of(z_ref[which] + c * KC, 8), KC)
            return pl.ds(c * KC, KC)

        def qk_chunk(g, qm, c, s_ref, m8):
            st = jnp.dot(k_ref[g, c * KC:(c + 1) * KC, :], qm, preferred_element_type=f32)
            s_ref[srows(c, 0), :] = st
            cm = jnp.max(st.reshape(KC // 8, 8, TQ), axis=0)
            return cm if m8 is None else jnp.maximum(m8, cm)

        def pv_chunk(h, c, s_ref, m, acc):
            p = jnp.exp2(s_ref[srows(c, 1), :] - m).astype(bf16)
            pv = jnp.dot(vt_ref[h, :, c * KC:(c + 1) * KC], p, preferred_element_type=f32)
            return pv if acc is None else acc + pv

        def finish(h, q0, acc):
            o = acc * (1.0 / acc[DH:DH + 1, :])
            ot_ref[pl.ds(pl.multiple_of(h * 32, 32), 32), pl.ds(q0, TQ)] = o.astype(bf16)

        def stage(nxt, cur, m, s_w, s_r):
            acc = None
            m8 = None
            if nxt is not None:
                qm = make_qm(*nxt)
            for c in range(NC):
                if nxt is not None:
                    m8 = qk_chunk(nxt[0], qm, c, s_w, m8)
                if cur is not None:
                    acc = pv_chunk(cur[0], c, s_r, m, acc)
            if cur is not None:
                finish(cur[0], cur[1], acc)
            if nxt is not None:
                return jnp.max(m8, axis=0, keepdims=True)
            return None

        def group_body(t, m, last):
            g = t % NG
            q0 = pl.multiple_of((t // NG) * TQ, TQ)
            bufs = (sa_ref, sb_ref)
            for j in range(4):
                if j < 3:
                    nxt = (g, j + 1, q0)
                elif last:
                    nxt = None
                else:
                    t1 = t + 1
                    nxt = (t1 % NG, 0, pl.multiple_of((t1 // NG) * TQ, TQ))
                m = stage(nxt, (g * 4 + j, q0), m, bufs[(j + 1) % 2], bufs[j % 2])
            return m

        if DO_ATT:
            m0 = stage((0, 0, 0), None, None, sa_ref, None)
            NT_ = NQ * NG
            m1 = lax.fori_loop(0, NT_ - 1, lambda t, m: group_body(t, m, False), m0)
            group_body(NT_ - 1, m1, True)
        else:
            ot_ref[...] = jnp.zeros_like(ot_ref)

        cp_wo.wait()
        wof = wo_ref[...].astype(f32)
        wop = jnp.concatenate(
            [blk for h in range(H) for blk in (wof[h * DH:(h + 1) * DH, :], zpad4)], axis=0)
        wot_ref[...] = wop.T.astype(bf16)
        cp_w1.wait(); cp_w3.wait(); cp_w2.wait()

        def out_copy(b):
            t0 = pl.multiple_of(b * TF, TF)
            return pltpu.make_async_copy(outb_ref.at[:, pl.ds(t0, TF)], out_hbm.at[:, pl.ds(t0, TF)], osems.at[b])

        def ffn_body(b, carry):
            t0 = pl.multiple_of(b * TF, TF)
            acc = jnp.dot(wot_ref[...], ot_ref[:, pl.ds(t0, TF)], preferred_element_type=f32)
            if DO_FFN:
                xq = xn_ref[pl.ds(t0, TF), :]
                for fc in range(F // FC):
                    fs = slice(fc * FC, (fc + 1) * FC)
                    gt = jnp.dot(xq, w1_ref[:, fs], preferred_element_type=f32)
                    up = jnp.dot(xq, w3_ref[:, fs], preferred_element_type=f32)
                    hh = (gt * jax.nn.sigmoid(gt) * up).astype(bf16)
                    acc = acc + lax.dot_general(w2t_ref[:, fs], hh, NT, preferred_element_type=f32)
            outb_ref[:, pl.ds(t0, TF)] = (xt_ref[:, pl.ds(t0, TF)].astype(f32) + acc).astype(bf16)
            out_copy(b).start()
            return carry
        lax.fori_loop(0, S // TF, ffn_body, 0)
        for b in range(S // TF):
            out_copy(b).wait()

    @jax.jit
    def fn(A_x, A_wqkv, A_wo, B_x, B_w1, B_w3, B_w2):
        xt = A_x.reshape(S, D).T
        w2t = B_w2.T
        anyspec = pl.BlockSpec(memory_space=pl.ANY)
        out = pl.pallas_call(
            kernel,
            in_specs=[anyspec] * 6,
            out_specs=anyspec,
            out_shape=jax.ShapeDtypeStruct((D, S), bf16),
            scratch_shapes=[
                pltpu.VMEM((D, S), bf16), pltpu.VMEM((D, 3 * D), bf16), pltpu.VMEM((D, D), bf16),
                pltpu.VMEM((D, F), bf16), pltpu.VMEM((D, F), bf16), pltpu.VMEM((D, F), bf16), pltpu.VMEM((D, S), bf16),
                pltpu.VMEM((3 * D, D), f32), pltpu.VMEM((D + 512, D), bf16), pltpu.VMEM((512, D), bf16), pltpu.VMEM((D, 512), bf16),
                pltpu.VMEM((S, D), bf16), pltpu.VMEM((NG, 128, S), bf16), pltpu.VMEM((NG, S, 128), bf16),
                pltpu.VMEM((H, 32, S), bf16), pltpu.VMEM((512, S), bf16),
                pltpu.VMEM((S, TQ), f32), pltpu.VMEM((S, TQ), f32),
                pltpu.SMEM((2,), jnp.int32), pltpu.SemaphoreType.DMA((6,)), pltpu.SemaphoreType.DMA((S // TF,))],
            compiler_params=pltpu.CompilerParams(vmem_limit_bytes=100 * 1024 * 1024),
            name="fusedk",
        )(xt, A_wqkv, A_wo, B_w1, B_w3, w2t)
        return out.T.reshape(1, S, D)
    return fn


_impl = build(KC=128, TF=512, OPAQUE=False)


@jax.jit
def pallas_parallel_sum__softmax_full_mha__glu_gated_swiglu__prompt_kernel(
    A_x: jax.Array,
    A_wqkv: jax.Array,
    A_wo: jax.Array,
    B_x: jax.Array,
    B_w1: jax.Array,
    B_w3: jax.Array,
    B_w2: jax.Array,
):
    return _impl(A_x, A_wqkv, A_wo, B_x, B_w1, B_w3, B_w2)
```

```python
import functools, math
import jax, jax.numpy as jnp
from jax import lax
from jax.experimental import pallas as pl
from jax.experimental.pallas import tpu as pltpu

S, D, H, DH, F = 2048, 448, 16, 28, 1792
NG, GW = 4, 112
EPS = 1e-5
QSCALE = (DH ** -0.5) * math.log2(math.e)
NT = (((1,), (1,)), ((), ()))
f32, bf16, u32 = jnp.float32, jnp.bfloat16, jnp.uint32


def build(TQ=512, TA=512, KC=128, TF=512, FC=256, LAG=2, NS=9, OW=128, OG=2, EX=1, RS=2, SPLIT0=384, PVFIRST=True, DEFER=True, FP0=8, FPS=32, FPD=4):
    NQ = S // TQ
    NC = S // KC
    NA = S // TA
    NI = NQ * H
    NO = S // OW
    NB = S // TF
    assert (NI - 1) % NS == 0 and NS % 3 == 0

    def kernel(xt_hbm, wqkv_hbm, wo_hbm, w1_hbm, w3_hbm, w2t_hbm, out_hbm,
               xt_ref, wqkv_ref, wo_ref, w1_ref, w3_ref, w2t_ref, outb_ref,
               wt_ref, wot_ref, xn_ref, xnt_ref, kt0_ref, qt_ref, k_ref, vt_ref, ot_ref, acc_ref,
               s0_ref, s1_ref, s2_ref, sems, osem):
        sbufs = (s0_ref, s1_ref, s2_ref)

        def ccopy(src, dst, c0, c1, k):
            return pltpu.make_async_copy(src.at[:, c0:c1], dst.at[:, c0:c1], sems.at[k])

        cp_x0 = ccopy(xt_hbm, xt_ref, 0, TA, 0)
        cp_wk = ccopy(wqkv_hbm, wqkv_ref, 384, 896, 1)
        cp_wq = ccopy(wqkv_hbm, wqkv_ref, 0, 384, 2)
        cp_wv = ccopy(wqkv_hbm, wqkv_ref, 896, 3 * D, 3)
        cp_x1 = ccopy(xt_hbm, xt_ref, TA, S, 4)
        cp_wo = pltpu.make_async_copy(wo_hbm, wo_ref, sems.at[5])
        cp_w1 = pltpu.make_async_copy(w1_hbm, w1_ref, sems.at[6])
        cp_w3 = pltpu.make_async_copy(w3_hbm, w3_ref, sems.at[7])
        cp_w2 = pltpu.make_async_copy(w2t_hbm, w2t_ref, sems.at[8])
        for cp in (cp_x0, cp_wk, cp_wq, cp_wv, cp_x1, cp_wo, cp_w1, cp_w3, cp_w2):
            cp.start()
        cp_x0.wait()

        def dsl(start, size, align):
            return pl.ds(start, size) if isinstance(start, int) else pl.ds(pl.multiple_of(start, align), size)

        def layernorm(c, store_xn=True):
            sl = dsl(c * TA, TA, TA)
            xt = xt_ref[:, sl].astype(f32)
            mu = jnp.sum(xt, axis=0, keepdims=True) * (1.0 / D)
            xc = xt - mu
            var = jnp.sum(xc * xc, axis=0, keepdims=True) * (1.0 / D)
            xnt = (xc * lax.rsqrt(var + EPS)).astype(bf16)
            if store_xn:
                xn_ref[sl, :] = xnt.T
                acc_ref[:, sl] = xt
            return xnt

        def proj(t0, xnt, p0, p1):
            n = xnt.shape[1]
            sl = dsl(t0, n, 128)
            zpad = jnp.zeros((128 - GW, n), f32)
            yy = jnp.dot(wt_ref[p0 * D:p1 * D, :], xnt, preferred_element_type=f32)
            for part in range(p0, p1):
                y = yy[(part - p0) * D:(part - p0 + 1) * D, :]
                if part == 0:
                    for g in range(NG):
                        kt = jnp.concatenate([y[GW * g:GW * (g + 1), :], zpad], axis=0)
                        k_ref[g, dsl(t0 // 2, n // 2, 64), :] = pltpu.bitcast(kt.astype(bf16).T, u32)
                elif part == 1:
                    yq = (y * QSCALE).astype(bf16)
                    for g in range(NG):
                        qt_ref[g, 0:GW // 2, sl] = pltpu.bitcast(yq[GW * g:GW * (g + 1), :], u32)
                        qt_ref[g, GW // 2:64, sl] = jnp.zeros((64 - GW // 2, n), u32)
                else:
                    vpad = jnp.where(lax.broadcasted_iota(jnp.int32, (32 - DH, n), 0) == 0, 1.0, 0.0).astype(f32)
                    for h in range(H):
                        vt_ref[h, :, sl] = pltpu.bitcast(jnp.concatenate([y[DH * h:DH * (h + 1), :], vpad], axis=0).astype(bf16), u32)

        xnt_ref[...] = layernorm(0, store_xn=False)
        cp_wk.wait()
        wt_ref[0:D, :] = wqkv_ref[:, 384:896].T[64:512, :]
        kt0_ref[...] = jnp.dot(wt_ref[0:D, :], xnt_ref[:, 0:SPLIT0], preferred_element_type=f32).astype(bf16)
        xn_ref[0:TA, :] = xnt_ref[...].T
        acc_ref[:, 0:TA] = xt_ref[:, 0:TA].astype(f32)
        cp_wq.wait()
        cp_wv.wait()
        if SPLIT0 < TA:
            proj(SPLIT0, xnt_ref[:, SPLIT0:TA], 0, 1)
        for g in range(NG):
            kt = jnp.concatenate([kt0_ref[GW * g:GW * (g + 1), :], jnp.zeros((128 - GW, SPLIT0), bf16)], axis=0)
            k_ref[g, 0:SPLIT0 // 2, :] = pltpu.bitcast(kt.T, u32)
        wt_ref[D:2 * D, :] = wqkv_ref[:, 0:512].T[0:D, :]
        wt_ref[2 * D:3 * D, :] = wqkv_ref[:, 896:3 * D].T
        proj(0, xnt_ref[...], 1, 2)
        cp_x1.wait()

        def a_body(c, carry):
            proj((c - 1) * TA, xnt_ref[...], 2, 3)
            xnt = layernorm(c)
            proj(c * TA, xnt, 0, 2)
            xnt_ref[...] = xnt
            return carry
        lax.fori_loop(1, NA, a_body, 0)
        cp_wo.wait()
        proj((NA - 1) * TA, xnt_ref[...], 2, 3)
        zpad4 = jnp.zeros((32 - DH, D), f32)
        wof = wo_ref[...].astype(f32)
        wop = jnp.concatenate(
            [blk for h in range(H) for blk in (wof[h * DH:(h + 1) * DH, :], zpad4)], axis=0)
        wot_ref[...] = wop.astype(bf16).T

        rowq = lax.broadcasted_iota(jnp.int32, (128, TQ), 0)

        def item(i):
            h = i % H
            return h, h // 4, h % 4, (i // H) * TQ

        def make_qm(g, j, q0):
            q = pltpu.bitcast(qt_ref[g, :, dsl(q0, TQ, TQ)], bf16)
            lo = j * DH
            return jnp.where((rowq >= lo) & (rowq < lo + DH), q.astype(f32), 0.0).astype(bf16)

        def qk_chunk(g, qm, c, s_ref, m8):
            r0, r1 = c * KC, (c + 1) * KC
            st = jnp.dot(pltpu.bitcast(k_ref[g, r0 // 2:r1 // 2, :], bf16), qm, preferred_element_type=f32)
            s_ref[r0:r1, :] = st
            cm = jnp.max(st.reshape(KC // 8, 8, TQ), axis=0)
            return cm if m8 is None else jnp.maximum(m8, cm)

        def pv_chunk(h, c, s_ref, m, acc):
            ks = slice(c * KC, (c + 1) * KC)
            p = jnp.exp2(s_ref[ks, :] - m).astype(bf16)
            pv = jnp.dot(pltpu.bitcast(vt_ref[h, :, ks], bf16), p, preferred_element_type=f32)
            return pv if acc is None else acc + pv

        def finish(i, acc):
            hc, _, _, qc = item(i)
            if DEFER:
                ot_ref[hc, :, dsl(qc, TQ, TQ)] = acc
            else:
                o = acc * (1.0 / acc[DH:DH + 1, :])
                ot_ref[dsl(hc * 32, 32, 32), dsl(qc, TQ, TQ)] = o.astype(bf16)

        def stage(i, s, m_prev, m_cur, acc, do_qk=True, do_pv=True, extra=None):
            m8 = None
            if do_qk:
                _, gn, jn, qn = item(i + 1)
                qm = make_qm(gn, jn, qn)
            ip = max(i - 1, 0) if isinstance(i, int) else jnp.maximum(i - 1, 0)
            for c in range(NC):
                if do_pv and PVFIRST:
                    acc = pv_step(i, ip, s, c, m_prev, m_cur, acc)
                if do_qk:
                    m8 = qk_chunk(gn, qm, c, sbufs[(s + 1) % 3], m8)
                if extra is not None:
                    extra(c)
                if do_pv and not PVFIRST:
                    acc = pv_step(i, ip, s, c, m_prev, m_cur, acc)
            m_next = jnp.max(m8, axis=0, keepdims=True) if do_qk else None
            return m_cur, m_next, acc

        def pv_step(i, ip, s, c, m_prev, m_cur, acc):
            if c < LAG:
                acc = pv_chunk(item(ip)[0], NC - LAG + c, sbufs[(s + 2) % 3], m_prev, acc)
                if c == LAG - 1:
                    finish(ip, acc)
                    acc = None
            else:
                acc = pv_chunk(item(i)[0], c - LAG, sbufs[s], m_cur, acc)
            return acc

        _, m0, _ = stage(-1, 2, None, None, None, do_pv=False)
        s1_ref[0:8, 0:128] = jnp.zeros((8, 128), f32)
        s2_ref[(NC - LAG) * KC:S, :] = jnp.zeros((LAG * KC, TQ), f32)

        cp_w1.wait(); cp_w3.wait(); cp_w2.wait()

        NIT = (NI - 1) // NS
        assert F // FC == NIT

        def att_body(t, carry):
            fs = dsl(t * FC, FC, FC)
            hstate = {}

            def ffn_up(b):
                xq = xn_ref[b * TF:(b + 1) * TF, :]
                gt = jnp.dot(xq, w1_ref[:, fs], preferred_element_type=f32)
                up = jnp.dot(xq, w3_ref[:, fs], preferred_element_type=f32)
                hstate[b] = (gt * jax.nn.sigmoid(gt) * up).astype(bf16)

            def ffn_down(b):
                tsl = slice(b * TF, (b + 1) * TF)
                acc_ref[:, tsl] += lax.dot_general(w2t_ref[:, fs], hstate.pop(b), NT, preferred_element_type=f32)

            sched = {}
            for b in range(NB):
                p = FP0 + b * FPS
                sched[p] = functools.partial(ffn_up, b)
                sched[p + FPD] = functools.partial(ffn_down, b)

            for s in range(NS):
                def extra(c, s=s):
                    fn_ = sched.get(s * NC + c)
                    if fn_ is not None:
                        fn_()
                carry = stage(t * NS + s, s % 3, *carry, extra=extra)
            return carry

        m_prev, m_cur, acc = lax.fori_loop(
            0, (NI - 1) // NS, att_body,
            (jnp.zeros((1, TQ), f32), m0, jnp.zeros((32, TQ), f32)))

        state = {"n": 0, "lo": 0}
        RH = D // RS

        def next_piece():
            b, r = divmod(state["n"], RS)
            sl = slice(b * OW, (b + 1) * OW)
            rs = slice(r * RH, (r + 1) * RH)
            if DEFER:
                if r == 0:
                    a = ot_ref[:, :, sl]
                    l = a[:, DH:DH + 1, :]
                    r0 = pl.reciprocal(l, approx=True)
                    r0 = r0 * (2.0 - l * r0)
                    state["o"] = (a * r0).reshape(H * 32, OW).astype(bf16)
                on = state["o"]
            else:
                on = ot_ref[:, sl]
            o = acc_ref[rs, sl] + jnp.dot(wot_ref[rs, :], on, preferred_element_type=f32)
            outb_ref[rs, sl] = o.astype(bf16)
            state["n"] += 1
            if r == RS - 1 and ((b + 1) % OG == 0 or b + 1 >= NO - 1):
                c0, c1 = state["lo"] * OW, (b + 1) * OW
                pltpu.make_async_copy(outb_ref.at[:, c0:c1], out_hbm.at[:, c0:c1], osem.at[0]).start()
                state["lo"] = b + 1

        def extra(c):
            if c % EX == 0 and state["n"] < RS * ((S - TQ) // OW):
                next_piece()
        sl_ = (NI - 1) % 3
        next_piece()
        _, _, acc = stage(NI - 1, sl_, m_prev, m_cur, acc, do_qk=False, extra=extra)
        for c in range(LAG):
            extra(c)
            acc = pv_chunk(H - 1, NC - LAG + c, sbufs[sl_], m_cur, acc)
        finish(NI - 1, acc)
        while state["n"] < NO * RS:
            next_piece()
        pltpu.make_async_copy(outb_ref, out_hbm, osem.at[0]).wait()

    @jax.jit
    def fn(A_x, A_wqkv, A_wo, B_x, B_w1, B_w3, B_w2):
        xt = A_x.reshape(S, D).T
        w2t = B_w2.T
        anyspec = pl.BlockSpec(memory_space=pl.ANY)
        out = pl.pallas_call(
            kernel,
            in_specs=[anyspec] * 6,
            out_specs=anyspec,
            out_shape=jax.ShapeDtypeStruct((D, S), bf16),
            scratch_shapes=[
                pltpu.VMEM((D, S), bf16), pltpu.VMEM((D, 3 * D), bf16), pltpu.VMEM((D, D), bf16),
                pltpu.VMEM((D, F), bf16), pltpu.VMEM((D, F), bf16), pltpu.VMEM((D, F), bf16), pltpu.VMEM((D, S), bf16),
                pltpu.VMEM((3 * D, D), bf16), pltpu.VMEM((D, 512), bf16),
                pltpu.VMEM((S, D), bf16), pltpu.VMEM((D, TA), bf16), pltpu.VMEM((D, SPLIT0), bf16),
                pltpu.VMEM((NG, 64, S), u32), pltpu.VMEM((NG, S // 2, 128), u32),
                pltpu.VMEM((H, 16, S), u32), pltpu.VMEM((H, 32, S), f32) if DEFER else pltpu.VMEM((512, S), bf16), pltpu.VMEM((D, S), f32),
                pltpu.VMEM((S, TQ), f32), pltpu.VMEM((S, TQ), f32), pltpu.VMEM((S, TQ), f32),
                pltpu.SemaphoreType.DMA((9,)), pltpu.SemaphoreType.DMA((1,))],
            compiler_params=pltpu.CompilerParams(vmem_limit_bytes=100 * 1024 * 1024),
            name="fusedk",
        )(xt, A_wqkv, A_wo, B_w1, B_w3, w2t)
        return out.T.reshape(1, S, D)
    return fn


_impl = build(FP0=0, FPS=36, FPD=4)


@jax.jit
def pallas_parallel_sum__softmax_full_mha__glu_gated_swiglu__prompt_kernel(
    A_x: jax.Array,
    A_wqkv: jax.Array,
    A_wo: jax.Array,
    B_x: jax.Array,
    B_w1: jax.Array,
    B_w3: jax.Array,
    B_w2: jax.Array,
):
    return _impl(A_x, A_wqkv, A_wo, B_x, B_w1, B_w3, B_w2)
```

```python
import functools, math
import jax, jax.numpy as jnp
from jax import lax
from jax.experimental import pallas as pl
from jax.experimental.pallas import tpu as pltpu

S, D, H, DH, F = 2048, 448, 16, 28, 1792
NG, GW = 4, 112
EPS = 1e-5
QSCALE = (DH ** -0.5) * math.log2(math.e)
NT = (((1,), (1,)), ((), ()))
f32, bf16, u32 = jnp.float32, jnp.bfloat16, jnp.uint32


def build(TQ=512, TA=512, KC=128, TF=512, FC=256, LAG=2, NS=9, OW=128, OG=2, EX=1, RS=2, SPLIT0=384,
          PVFIRST=True, FPOS=(0, 40, 80, 138), FPD=4, NOFF=160, NCH=2, GATE=0, TANH=True,
          ASSIGN=((0, 1), (2, 3), (4, 5), (6, 7, 8)), AHEAD=3, INFL=0, LATIN=True, WG=1024, WU=1024, WD=896, SKIP=0, KBL=True, TR=(8, 5, 2), AEVERY=1, NKB=8, BG=(3,), BU=(3,), BD=(3,), ALAST=138, BC=(18, 24, 14), BSKIP=20, RELB=4, SELTIE=False, TR2=(), TR2E=2, RELR=1, LOWC=(), TRL=(6, 2)):
    NQ = S // TQ
    NC = S // KC
    NA = S // TA
    NI = NQ * H
    NO = S // OW
    NB = S // TF
    NTL = TQ // 128
    assert (NI - 1) % NS == 0 and NS % 3 == 0
    assert NOFF % 16 == 0 and NOFF <= 16 * NC
    nshort = NOFF // 16
    QR = []
    r_ = NOFF
    for c_ in range(NC):
        short = ((c_ + 1) * nshort) // NC - (c_ * nshort) // NC
        QR.append((r_, r_ + KC - 16 * short))
        r_ = QR[-1][1]
    assert r_ == S

    def kernel(xt_hbm, wqkv_hbm, wo_hbm, w1_hbm, w3_hbm, w2t_hbm, out_hbm,
               xt_ref, wqkv_ref, wo_ref, wf_ref, outb_ref,
               wt_ref, wot_ref, xn_ref, xnt_ref, kt0_ref, qt_ref, k_ref, vt_ref, ot_ref, acc_ref,
               qf_ref, so_ref, kb_ref, ko_ref,
               s0_ref, s1_ref, s2_ref, sems, osem):
        sbufs = (s0_ref, s1_ref, s2_ref)

        def ccopy(src, dst, c0, c1, k):
            return pltpu.make_async_copy(src.at[:, c0:c1], dst.at[:, c0:c1], sems.at[k])

        cp_x0 = ccopy(xt_hbm, xt_ref, 0, TA, 0)
        cp_wk = ccopy(wqkv_hbm, wqkv_ref, 384, 896, 1)
        cp_wq = ccopy(wqkv_hbm, wqkv_ref, 0, 384, 2)
        cp_wv = ccopy(wqkv_hbm, wqkv_ref, 896, 3 * D, 3)
        cp_x1 = ccopy(xt_hbm, xt_ref, TA, S, 4)
        cp_wo = pltpu.make_async_copy(wo_hbm, wo_ref, sems.at[5])
        for cp in (cp_x0, cp_wk, cp_wq, cp_wv, cp_x1, cp_wo):
            cp.start()
        cp_x0.wait()

        def dsl(start, size, align):
            return pl.ds(start, size) if isinstance(start, int) else pl.ds(pl.multiple_of(start, align), size)

        def layernorm(c, store_xn=True):
            sl = dsl(c * TA, TA, TA)
            xt = xt_ref[:, sl].astype(f32)
            mu = jnp.sum(xt, axis=0, keepdims=True) * (1.0 / D)
            xc = xt - mu
            var = jnp.sum(xc * xc, axis=0, keepdims=True) * (1.0 / D)
            xnt = (xc * lax.rsqrt(var + EPS)).astype(bf16)
            if store_xn:
                xn_ref[sl, :] = xnt.T
                acc_ref[:, sl] = xt
            return xnt

        def proj(t0, xnt, p0, p1):
            n = xnt.shape[1]
            sl = dsl(t0, n, 128)
            zpad = jnp.zeros((128 - GW, n), f32)
            yy = jnp.dot(wt_ref[p0 * D:p1 * D, :], xnt, preferred_element_type=f32)
            for part in range(p0, p1):
                y = yy[(part - p0) * D:(part - p0 + 1) * D, :]
                if part == 0:
                    for g in range(NG):
                        kt = jnp.concatenate([y[GW * g:GW * (g + 1), :], zpad], axis=0)
                        k_ref[g, dsl(t0 // 2, n // 2, 64), :] = pltpu.bitcast(kt.astype(bf16).T, u32)
                elif part == 1:
                    yq = (y * QSCALE).astype(bf16)
                    if NOFF:
                        yf = yq.astype(f32)
                        for h in range(H):
                            yh = yf[h * DH:(h + 1) * DH, :]
                            for t in range(n // 128):
                                qf_ref[(t0 // 128 + t) * H + h, 0:DH, :] = yh[:, t * 128:(t + 1) * 128]
                    for g in range(NG):
                        qt_ref[g, 0:GW // 2, sl] = pltpu.bitcast(yq[GW * g:GW * (g + 1), :], u32)
                        qt_ref[g, GW // 2:64, sl] = jnp.zeros((64 - GW // 2, n), u32)
                else:
                    vpad = jnp.where(lax.broadcasted_iota(jnp.int32, (32 - DH, n), 0) == 0, 1.0, 0.0).astype(f32)
                    for h in range(H):
                        vt_ref[h, :, sl] = pltpu.bitcast(
                            jnp.concatenate([y[DH * h:DH * (h + 1), :], vpad], axis=0).astype(bf16), u32)

        def head_k(h, rel=None):
            kp = ko_ref[h // 4]
            if rel is not None:
                z = pltpu.bitcast(rel - rel, u32)
                kp = kp | jnp.concatenate([z] * (NOFF // 16), axis=0)
            j = h % 4
            if isinstance(j, int):
                if j:
                    kp = pltpu.roll(kp, 128 - DH * j, 1)
            else:
                kp = pltpu.roll(kp, (128 - DH * j) % 128, 1)
            return pltpu.bitcast(kp, bf16).astype(f32)

        def build_col(kf, slot, d):
            bc = jnp.broadcast_to(kf[:, d:d + 1], (NOFF, 128))
            for kg in range(NOFF // 8):
                kb_ref[slot, (kg * DH + d) * 8:(kg * DH + d + 1) * 8, :] = bc[kg * 8:(kg + 1) * 8, :]
            return bc[NOFF - 8:NOFF, :]

        def build_head(h):
            kf = head_k(h)
            for d in range(DH):
                build_col(kf, h % NKB, d)

        for k, src in enumerate((w1_hbm, w3_hbm, w2t_hbm)):
            for j in range(F // FC):
                pltpu.make_async_copy(src.at[:, j * FC:(j + 1) * FC], wf_ref.at[k, j], sems.at[6]).start()
        xnt_ref[...] = layernorm(0, store_xn=False)
        cp_wk.wait()
        wt_ref[0:D, :] = wqkv_ref[:, 384:896].T[64:512, :]
        kt0_ref[...] = jnp.dot(wt_ref[0:D, :], xnt_ref[:, 0:SPLIT0], preferred_element_type=f32).astype(bf16)
        xn_ref[0:TA, :] = xnt_ref[...].T
        acc_ref[:, 0:TA] = xt_ref[:, 0:TA].astype(f32)
        cp_wq.wait()
        cp_wv.wait()
        if SPLIT0 < TA:
            proj(SPLIT0, xnt_ref[:, SPLIT0:TA], 0, 1)
        for g in range(NG):
            kt = jnp.concatenate([kt0_ref[GW * g:GW * (g + 1), :], jnp.zeros((128 - GW, SPLIT0), bf16)], axis=0)
            kp = pltpu.bitcast(kt.T, u32)
            k_ref[g, 0:SPLIT0 // 2, :] = kp
            ko_ref[g] = kp[0:NOFF // 2, :]
        wt_ref[D:2 * D, :] = wqkv_ref[:, 0:512].T[0:D, :]
        wt_ref[2 * D:3 * D, :] = wqkv_ref[:, 896:3 * D].T
        proj(0, xnt_ref[...], 1, 2)
        cp_x1.wait()

        def a_body(c, carry):
            proj((c - 1) * TA, xnt_ref[...], 2, 3)
            xnt = layernorm(c)
            proj(c * TA, xnt, 0, 2)
            xnt_ref[...] = xnt
            build_head(c)
            return carry
        lax.fori_loop(1, NA, a_body, 0)
        cp_wo.wait()
        build_head(4)
        proj((NA - 1) * TA, xnt_ref[...], 2, 3)
        zpad4 = jnp.zeros((32 - DH, D), f32)
        wof = wo_ref[...].astype(f32)
        wop = jnp.concatenate(
            [blk for h in range(H) for blk in (wof[h * DH:(h + 1) * DH, :], zpad4)], axis=0)
        wot_ref[...] = wop.astype(bf16).T

        rowq = lax.broadcasted_iota(jnp.int32, (128, TQ), 0)

        def item(i):
            h = i // NQ
            return h, h // 4, h % 4, (i % NQ) * TQ

        def make_qm(g, j, q0):
            q = pltpu.bitcast(qt_ref[g, :, dsl(q0, TQ, TQ)], bf16)
            lo = j * DH
            return jnp.where((rowq >= lo) & (rowq < lo + DH), q.astype(f32), 0.0).astype(bf16)

        def rmax(st, m8):
            cm = jnp.max(st.reshape(st.shape[0] // 8, 8, TQ), axis=0)
            return cm if m8 is None else jnp.maximum(m8, cm)

        def qk_rows(g, qm, r0, r1):
            return jnp.dot(pltpu.bitcast(k_ref[g, r0 // 2:r1 // 2, :], bf16), qm, preferred_element_type=f32)

        SO0 = 0

        def so_rows(slot, t, r0, n):
            base = SO0 + (slot * NTL + t) * NOFF + r0
            return slice(base, base + n)

        def so_load(slot, k0, k1):
            return jnp.concatenate([so_ref[so_rows(slot, t, k0, k1 - k0), :] for t in range(NTL)], axis=1)

        def so_store(slot, val):
            for t in range(NTL):
                so_ref[so_rows(slot, t, 0, NOFF), :] = val[:, t * 128:(t + 1) * 128]

        pending = []

        def vpu_flush(keep):
            while len(pending) > keep:
                rows, val = pending.pop(0)
                qf_ref[rows, :] = val

        def vpu_chain(h, q0, kg, t, slot):
            r0 = kg * 8
            accs = [None] * NCH
            qi = (q0 // 128 + t) * H + h
            for d in range(DH):
                kb = kb_ref[h % NKB, (kg * DH + d) * 8:(kg * DH + d + 1) * 8, :]
                qb = qf_ref[qi, pl.ds(d, 8, stride=0), :]
                p = kb * qb
                accs[d % NCH] = p if accs[d % NCH] is None else accs[d % NCH] + p
            acc = accs[0]
            for a_ in accs[1:]:
                acc = acc + a_
            so_ref[so_rows(slot, t, r0, 8), :] = acc
            return acc

        def pv_chunk(h, c, s_ref, slot, m, acc):
            ks = slice(c * KC, (c + 1) * KC)
            k0, k1 = c * KC, (c + 1) * KC
            parts = []
            if k0 < NOFF:
                parts.append(so_load(slot, k0, min(k1, NOFF)))
            if k1 > NOFF:
                parts.append(s_ref[max(k0, NOFF):k1, :])
            sv = parts[0] if len(parts) == 1 else jnp.concatenate(parts, axis=0)
            p = jnp.exp2(sv - m).astype(bf16)
            pv = jnp.dot(pltpu.bitcast(vt_ref[h, :, ks], bf16), p, preferred_element_type=f32)
            return pv if acc is None else acc + pv

        def finish(i, acc):
            hc, _, _, qc = item(i)
            ot_ref[hc, :, dsl(qc, TQ, TQ)] = acc

        def pv_step(i, ip, s, c, m_prev, m_cur, acc):
            if c < LAG:
                acc = pv_chunk(item(ip)[0], NC - LAG + c, sbufs[(s + 2) % 3], None, m_prev, acc)
                if c == LAG - 1:
                    finish(ip, acc)
                    acc = None
            else:
                acc = pv_chunk(item(i)[0], c - LAG, sbufs[s % 3], (s - 1) % NS, m_cur, acc)
            return acc

        def stage(i, s, m_prev, m_cur, acc, do_qk=True, do_pv=True, extra=None, full_qk=False, tie_qk=None):
            m8 = None
            if do_qk:
                _, gn, jn, qn = item(i + 1)
                qm = make_qm(gn, jn, qn)
            ip = max(i - 1, 0) if isinstance(i, int) else jnp.maximum(i - 1, 0)
            s_w = sbufs[(s + 1) % 3]
            for c in range(NC):
                if do_pv and PVFIRST:
                    acc = pv_step(i, ip, s, c, m_prev, m_cur, acc)
                if do_qk:
                    r0, r1 = QR[c]
                    if c == 0 and NOFF and full_qk:
                        so_store(s % NS, qk_rows(gn, qm, 0, NOFF))
                    st = qk_rows(gn, qm, r0, r1)
                    if tie_qk is not None:
                        st = tie_qk(st, s * NC + c)
                    s_w[r0:r1, :] = st
                    m8 = rmax(st, m8)
                    o0, o1 = ((c * NOFF // 8) // NC) * 8, (((c + 1) * NOFF // 8) // NC) * 8
                    if o1 > o0:
                        m8 = rmax(so_load(s % NS, o0, o1), m8)
                if extra is not None:
                    extra(c)
                if do_pv and not PVFIRST:
                    acc = pv_step(i, ip, s, c, m_prev, m_cur, acc)
            m_next = None
            if do_qk:
                m_next = jnp.max(m8, axis=0, keepdims=True)
            return m_cur, m_next, acc

        _, m0, _ = stage(-1, NS - 1, None, None, None, do_pv=False, full_qk=True)
        if NOFF:
            for s_ in range(AHEAD):
                _, g_, j_, q_ = item(s_ + 1)
                so_store(s_, qk_rows(g_, make_qm(g_, j_, q_), 0, NOFF))
        s1_ref[0:8, 0:128] = jnp.zeros((8, 128), f32)
        s2_ref[(NC - LAG) * KC:S, :] = jnp.zeros((LAG * KC, TQ), f32)

        pltpu.make_async_copy(wf_ref, wf_ref, sems.at[6]).wait()

        NIT = (NI - 1) // NS
        assert F // FC == NIT

        def att_body(t, carry):
            never = lax.broadcasted_iota(jnp.int32, (8, 128), 0) < jnp.minimum(t, 0)

            def tied(v, res):
                return jnp.where(never, res, v) if SELTIE else v + (res - res)

            hstate = {}

            jobs = []
            if NOFF:
                for s in range(NS):
                    i1 = jnp.minimum(t * NS + s + AHEAD + 1, NI - 1)
                    hh, _, _, q0 = item(i1)
                    for kb_ in range(NOFF // 8):
                        for tt in range(NTL):
                            kg = (kb_ // NTL) * NTL + (kb_ + tt) % NTL if LATIN else kb_
                            jobs.append((hh, q0, kg, tt, (s + AHEAD) % NS))
            att_steps = [n for n in range(NS * NC) if n % AEVERY == 0 and n <= ALAST]
            trs = {n: (TRL if n % NC in LOWC else (TR2 if (TR2 and n % TR2E == 0) else TR)) for n in att_steps}
            n_att = sum(len(v) for v in trs.values())
            n_ffn = max(len(jobs) - n_att, 0)
            total = NB * (WG + WU + WD) - len(BG) * WG - len(BU) * WU - len(BD) * WD
            st_ = {"time": 0, "fdone": 0, "done": 0}

            def tie_at(y, pos):
                R, C = y.shape[0] // 8, y.shape[1] // 128
                cols = [[None] * R for _ in range(C)]
                for c in range(C):
                    for r in range(R):
                        cols[c][r] = y[r * 8:(r + 1) * 8, c * 128:(c + 1) * 128]
                for (r, c) in pos:
                    if st_["done"] < len(jobs):
                        res = vpu_chain(*jobs[st_["done"]])
                        st_["done"] += 1
                        cols[c][r] = tied(cols[c][r], res)
                return jnp.concatenate([jnp.concatenate(col, axis=0) for col in cols], axis=1)

            def tie(y, w):
                st_["time"] += w
                want = (n_ffn * st_["time"]) // total
                n = want - st_["fdone"]
                st_["fdone"] = want
                if n == 0:
                    return y
                R, C = y.shape[0] // 8, y.shape[1] // 128
                idx = [((k + 1) * R * C) // n - 1 for k in range(n)]
                return tie_at(y, [(i_ % R, i_ // R) for i_ in idx])

            def tie_qk(st, n):
                if n == ALAST:
                    bst["rel"] = st[0:8, 0:128]
                if n in att_steps:
                    return tie_at(st, [(st.shape[0] // 8 - r, k % NTL) for k, r in enumerate(trs[n])])
                return st

            bst = {"n": 0}

            def tie_build(y, ncols, skip):
                R, C = y.shape[0] // 8, y.shape[1] // 128
                cols = [[y[r * 8:(r + 1) * 8, c * 128:(c + 1) * 128] for r in range(R)] for c in range(C)]
                lo = (R * C * skip) // 100
                for n in range(ncols):
                    k_, d = divmod(bst["n"], DH)
                    bst["n"] += 1
                    hb = 5 + 2 * t + k_
                    if d == 0:
                        bst["kf"] = head_k(jnp.minimum(hb, H - 1), bst["rel"])
                    res = build_col(bst["kf"], hb % NKB, d)
                    i_ = lo + ((n + 1) * (R * C - lo)) // ncols - 1
                    cols[i_ // R][i_ % R] = tied(cols[i_ // R][i_ % R], res)
                    if d == DH - RELB:
                        bst["rel"] = cols[i_ // R][i_ % R]
                return jnp.concatenate([jnp.concatenate(col, axis=0) for col in cols], axis=1)

            def ffn_up(b):
                xq = xn_ref[b * TF:(b + 1) * TF, :]
                gt = jnp.dot(xq, wf_ref[0, t], preferred_element_type=f32)
                gt = tie_build(gt, BC[0], BSKIP) if b in BG else tie(gt, WG)
                if b in BU and b not in BG:
                    bst["rel"] = gt[TF - RELR * 8:TF - RELR * 8 + 8, FC - 128:FC]
                up = jnp.dot(xq, wf_ref[1, t], preferred_element_type=f32)
                up = tie_build(up, BC[1], 0 if b in BG else BSKIP) if b in BU else tie(up, WU)
                if TANH:
                    sg = 0.5 * jnp.tanh(0.5 * gt) + 0.5
                else:
                    sg = jax.nn.sigmoid(gt)
                hstate[b] = (gt * up * sg).astype(bf16)

            def ffn_down(b):
                tsl = slice(b * TF, (b + 1) * TF)
                dn = lax.dot_general(wf_ref[2, t], hstate.pop(b), NT, preferred_element_type=f32)
                acc_ref[:, tsl] += (tie_build(dn, BC[2], 0) if BC[2] else dn) if b in BD else tie(dn, WD)

            sched = {}
            for b in range(NB):
                sched[FPOS[b]] = functools.partial(ffn_up, b)
                sched[FPOS[b] + FPD] = functools.partial(ffn_down, b)

            for s in range(NS):
                def extra(c, s=s):
                    fn_ = sched.get(s * NC + c)
                    if fn_ is not None:
                        fn_()
                carry = stage(t * NS + s, s, *carry, extra=extra, tie_qk=tie_qk)
            assert st_['done'] == len(jobs), (st_, len(jobs))
            return carry

        m_prev, m_cur, acc = lax.fori_loop(
            0, NIT, att_body,
            (jnp.zeros((1, TQ), f32), m0, jnp.zeros((32, TQ), f32)))

        state = {"n": 0, "lo": 0}
        RH = D // RS

        def next_piece():
            b, r = divmod(state["n"], RS)
            sl = slice(b * OW, (b + 1) * OW)
            rs = slice(r * RH, (r + 1) * RH)
            if r == 0:
                a = ot_ref[:, :, sl]
                l = a[:, DH:DH + 1, :]
                r0 = pl.reciprocal(l, approx=True)
                r0 = r0 * (2.0 - l * r0)
                state["o"] = (a * r0).reshape(H * 32, OW).astype(bf16)
            o = acc_ref[rs, sl] + jnp.dot(wot_ref[rs, :], state["o"], preferred_element_type=f32)
            outb_ref[rs, sl] = o.astype(bf16)
            state["n"] += 1
            if r == RS - 1 and ((b + 1) % OG == 0 or b + 1 >= NO - 1):
                c0, c1 = state["lo"] * OW, (b + 1) * OW
                pltpu.make_async_copy(outb_ref.at[:, c0:c1], out_hbm.at[:, c0:c1], osem.at[0]).start()
                state["lo"] = b + 1

        def extra(c):
            if c % EX == 0 and state["n"] < RS * ((S - 2 * TQ) // OW):
                next_piece()
        next_piece()
        _, _, acc = stage(NI - 1, 0, m_prev, m_cur, acc, do_qk=False, extra=extra)
        for c in range(LAG):
            next_piece()
            acc = pv_chunk(H - 1, NC - LAG + c, sbufs[0], None, m_cur, acc)
        finish(NI - 1, acc)
        while state["n"] < NO * RS:
            next_piece()
        pltpu.make_async_copy(outb_ref, out_hbm, osem.at[0]).wait()

    @jax.jit
    def fn(A_x, A_wqkv, A_wo, B_x, B_w1, B_w3, B_w2):
        xt = A_x.reshape(S, D).T
        w2t = B_w2.T
        anyspec = pl.BlockSpec(memory_space=pl.ANY)
        no = max(NOFF, 8)
        out = pl.pallas_call(
            kernel,
            in_specs=[anyspec] * 6,
            out_specs=anyspec,
            out_shape=jax.ShapeDtypeStruct((D, S), bf16),
            scratch_shapes=[
                pltpu.VMEM((D, S), bf16), pltpu.VMEM((D, 3 * D), bf16), pltpu.VMEM((D, D), bf16),
                pltpu.VMEM((3, F // FC, D, FC), bf16), pltpu.VMEM((D, S), bf16),
                pltpu.VMEM((3 * D, D), bf16), pltpu.VMEM((D, 512), bf16),
                pltpu.VMEM((S, D), bf16), pltpu.VMEM((D, TA), bf16), pltpu.VMEM((D, SPLIT0), bf16),
                pltpu.VMEM((NG, 64, S), u32), pltpu.VMEM((NG, S // 2, 128), u32),
                pltpu.VMEM((H, 16, S), u32), pltpu.VMEM((H, 32, S), f32), pltpu.VMEM((D, S), f32),
                pltpu.VMEM(((S // 128) * H, 32, 128), f32), pltpu.VMEM((NS * NTL * no, 128), f32), pltpu.VMEM((NKB, DH * no, 128), f32), pltpu.VMEM((NG, no // 2, 128), u32),
                pltpu.VMEM((S, TQ), f32), pltpu.VMEM((S, TQ), f32), pltpu.VMEM((S, TQ), f32),
                pltpu.SemaphoreType.DMA((9,)), pltpu.SemaphoreType.DMA((1,))],
            compiler_params=pltpu.CompilerParams(vmem_limit_bytes=110 * 1024 * 1024),
            name="fusedk",
        )(xt, A_wqkv, A_wo, B_w1, B_w3, w2t)
        return out.T.reshape(1, S, D)
    return fn


_impl = build(TR=(7,4,1))


@jax.jit
def pallas_parallel_sum__softmax_full_mha__glu_gated_swiglu__prompt_kernel(
    A_x: jax.Array,
    A_wqkv: jax.Array,
    A_wo: jax.Array,
    B_x: jax.Array,
    B_w1: jax.Array,
    B_w3: jax.Array,
    B_w2: jax.Array,
):
    return _impl(A_x, A_wqkv, A_wo, B_x, B_w1, B_w3, B_w2)
```

```python
import functools, math
import jax, jax.numpy as jnp
from jax import lax
from jax.experimental import pallas as pl
from jax.experimental.pallas import tpu as pltpu

S, D, H, DH, F = 2048, 448, 16, 28, 1792
NG, GW, HD = 4, 112, 224
EPS = 1e-5
QSCALE = (DH ** -0.5) * math.log2(math.e)
NT = (((1,), (1,)), ((), ()))
f32, bf16, u32 = jnp.float32, jnp.bfloat16, jnp.uint32
BIG = 2.0 ** 110


def build(NOFF=224, TR=(13, 10, 7, 4, 1), TR2=(), TR2E=2, LAG=3, AHEAD=3, FPOS=(0, 40, 80, 138), FPD=4, ALAST=138,
          WG=1024, WU=1024, WD=896, BG=(3,), BC=(18, 24, 14), BSKIP=20, RELB=4, LATIN=False,
          PREP0=5, FALLBACK=True, FORCE=False, OA=64, DSKIP=0, LOWO=(), TRL=(10, 4), SELTIE=0):
    TQ = TA = TF = 512
    KC, FC, OW, OG, RS, SPLIT0, NS, NKB = 128, 256, 128, 2, 2, 384, 9, 8
    NQ, NC, NA, NB, NO, NTL = S // TQ, S // KC, S // TA, S // TF, S // OW, TQ // 128
    NI = NQ * H
    NIT = (NI - 1) // NS
    NKG = NOFF // 8
    assert NOFF % 16 == 0 and F // FC == NIT
    def _pat(n):
        return [16 * (((c_ + 1) * (n // 16)) // 4 - (c_ * (n // 16)) // 4) for c_ in range(4)]
    OFFR = _pat(OA) * 3 + _pat(NOFF - 3 * OA)
    OFFS = [sum(OFFR[:c_]) for c_ in range(NC + 1)]
    assert OFFS[NC] == NOFF

    def kernel(xt_hbm, wqkv_hbm, wo_hbm, w1_hbm, w3_hbm, w2t_hbm, out_hbm,
               xt_ref, wqkv_ref, wo_ref, wf_ref, outb_ref,
               wt_ref, wot_ref, xn_ref, xnt_ref, kt0_ref, qt_ref, k_ref, vt_ref, ot_ref, acc_ref,
               qf_ref, so_ref, mo_ref, kb_ref, ko_ref, p_ref, s_ref, sems, osem):

        def ccopy(src, dst, c0, c1, k):
            return pltpu.make_async_copy(src.at[:, c0:c1], dst.at[:, c0:c1], sems.at[k])

        cp_x0 = ccopy(xt_hbm, xt_ref, 0, TA, 0)
        cp_wk = ccopy(wqkv_hbm, wqkv_ref, 384, 896, 1)
        cp_wq = ccopy(wqkv_hbm, wqkv_ref, 0, 384, 2)
        cp_wv = ccopy(wqkv_hbm, wqkv_ref, 896, 3 * D, 3)
        cp_x1 = ccopy(xt_hbm, xt_ref, TA, S, 4)
        cp_wo = pltpu.make_async_copy(wo_hbm, wo_ref, sems.at[5])
        for cp in (cp_x0, cp_wk, cp_wq, cp_wv, cp_x1, cp_wo):
            cp.start()
        acc_ref[...] = jnp.zeros((D, S), f32)
        cp_x0.wait()
        for k, src in enumerate((w1_hbm, w3_hbm, w2t_hbm)):
            for j in range(NIT):
                pltpu.make_async_copy(src.at[:, j * FC:(j + 1) * FC], wf_ref.at[k, j], sems.at[6]).start()

        def dsl(start, size, align):
            return pl.ds(start, size) if isinstance(start, int) else pl.ds(pl.multiple_of(start, align), size)

        def first_row(n_rows, n, dtype):
            return jnp.where(lax.broadcasted_iota(jnp.int32, (n_rows, n), 0) == 0, 1.0, 0.0).astype(dtype)

        def layernorm(c, store=True):
            sl = dsl(c * TA, TA, TA)
            xt = xt_ref[:, sl].astype(f32)
            mu = jnp.sum(xt, axis=0, keepdims=True) * (1.0 / D)
            xc = xt - mu
            var = jnp.sum(xc * xc, axis=0, keepdims=True) * (1.0 / D)
            xnt = (xc * lax.rsqrt(var + EPS)).astype(bf16)
            if store:
                xn_ref[dsl(c * (TA // 2), TA // 2, TA // 2), :] = pltpu.bitcast(xnt.T, u32)
            return xnt

        def pack_k(kt):
            n = kt.shape[1]
            return pltpu.bitcast(jnp.concatenate([kt, first_row(128 - GW, n, bf16)], axis=0).T, u32)

        def proj(t0, xnt, p0, p1):
            n = xnt.shape[1]
            sl = dsl(t0, n, 128)
            yy = jnp.dot(pltpu.bitcast(wt_ref[p0 * HD:p1 * HD, :], bf16), xnt, preferred_element_type=f32)
            for part in range(p0, p1):
                y = yy[(part - p0) * D:(part - p0 + 1) * D, :]
                if part == 0:
                    yk = y.astype(bf16)
                    for g in range(NG):
                        k_ref[g, dsl(t0 // 2, n // 2, 64), :] = pack_k(yk[GW * g:GW * (g + 1), :])
                elif part == 1:
                    yq = (y * QSCALE).astype(bf16)
                    yf = yq.astype(f32)
                    for h in range(H):
                        yh = yf[h * DH:(h + 1) * DH, :]
                        for t in range(n // 128):
                            qf_ref[(t0 // 128 + t) * H + h, 0:DH, :] = yh[:, t * 128:(t + 1) * 128]
                    for g in range(NG):
                        qt_ref[g, :, sl] = pltpu.bitcast(yq[GW * g:GW * (g + 1), :], u32)
                else:
                    vpad = first_row(32 - DH, n, f32)
                    for h in range(H):
                        vt_ref[h, :, sl] = pltpu.bitcast(
                            jnp.concatenate([y[DH * h:DH * (h + 1), :], vpad], axis=0).astype(bf16), u32)

        def head_k(kp, h, rel=None):
            if rel is not None:
                z = pltpu.bitcast(rel - rel, u32)
                kp = kp | jnp.concatenate([z] * (kp.shape[0] // 8), axis=0)
            kp = pltpu.roll(kp, (128 - DH * (h % 4)) % 128, 1)
            return pltpu.bitcast(kp, bf16).astype(f32)

        def build_col(kf, slot, kgs, d):
            n = kf.shape[0]
            bc = jnp.broadcast_to(kf[:, d:d + 1], (n, 128))
            kb_ref[slot, kgs, d * 8:(d + 1) * 8, :] = bc.reshape(n // 8, 8, 128)
            return bc[n - 8:n, :]

        def gather_keys(c, pat):
            n = sum(pat)
            out = []
            for g in range(NG):
                kp = jnp.concatenate([k_ref[g, dsl(c * (TA // 2) + j * 64, r // 2, 8), :]
                                      for j, r in enumerate(pat) if r], axis=0)
                ko_ref[g, dsl(c * (OA // 2), n // 2, 8), :] = kp
                out.append(kp)
            return out

        def prebuild(c, kps):
            n = 2 * kps[0].shape[0]
            for h in range(1, 5):
                kf = head_k(kps[h // 4], h)
                for d in range(DH):
                    build_col(kf, h, pl.ds(c * (OA // 8), n // 8), d)

        def xnt_load(c0=0, c1=TA):
            return pltpu.bitcast(xnt_ref[:, c0:c1], bf16)

        xnt_ref[...] = pltpu.bitcast(layernorm(0, store=False), u32)
        cp_wk.wait()
        wt_ref[0:HD, :] = pltpu.bitcast(wqkv_ref[:, 384:896].T[64:512, :], u32)
        kt0_ref[...] = pltpu.bitcast(jnp.dot(pltpu.bitcast(wt_ref[0:HD, :], bf16), xnt_load(0, SPLIT0),
                                             preferred_element_type=f32).astype(bf16), u32)
        xn_ref[0:TA // 2, :] = pltpu.bitcast(xnt_load().T, u32)
        cp_wq.wait()
        cp_wv.wait()
        proj(SPLIT0, xnt_load(SPLIT0, TA), 0, 1)
        for g in range(NG):
            k_ref[g, 0:SPLIT0 // 2, :] = pack_k(pltpu.bitcast(kt0_ref[GW // 2 * g:GW // 2 * (g + 1), :], bf16))
        wt_ref[HD:2 * HD, :] = pltpu.bitcast(wqkv_ref[:, 0:512].T[0:D, :], u32)
        wt_ref[2 * HD:3 * HD, :] = pltpu.bitcast(wqkv_ref[:, 896:3 * D].T, u32)
        proj(0, xnt_load(), 1, 2)
        cp_x1.wait()

        def a_body(c, carry):
            kps = gather_keys(c - 1, OFFR[0:4])
            proj((c - 1) * TA, xnt_load(), 2, 3)
            xnt = layernorm(c)
            proj(c * TA, xnt, 0, 2)
            xnt_ref[...] = pltpu.bitcast(xnt, u32)
            prebuild(c - 1, kps)
            return carry
        lax.fori_loop(1, NA, a_body, 0)
        cp_wo.wait()

        rowq = lax.broadcasted_iota(jnp.int32, (GW // 2, TQ), 0)
        row16 = lax.broadcasted_iota(jnp.int32, (128 - GW, TQ), 0)

        def item(i):
            h = i // NQ
            return h, h // 4, h % 4, (i % NQ) * TQ

        def make_qm(i, cneg):
            _, g, j, q0 = item(i)
            lo = j * (DH // 2)
            qm = jnp.where((rowq >= lo) & (rowq < lo + DH // 2), qt_ref[g, :, dsl(q0, TQ, TQ)], jnp.uint32(0))
            if cneg is None:
                tail = jnp.zeros((64 - GW // 2, TQ), u32)
            else:
                tail = pltpu.bitcast(jnp.where(row16 == 0, cneg, 0.0).astype(bf16), u32)
            return pltpu.bitcast(jnp.concatenate([qm, tail], axis=0), bf16)

        def qk_rows(g, qm, r0, r1):
            return jnp.dot(pltpu.bitcast(k_ref[g, r0 // 2:r1 // 2, :], bf16), qm, preferred_element_type=f32)

        def so_load(slot, k0, k1):
            return jnp.concatenate([so_ref[slot * NTL + t, k0:k1, :] for t in range(NTL)], axis=1)

        def so_store(slot, val):
            for t in range(NTL):
                so_ref[slot * NTL + t] = val[:, t * 128:(t + 1) * 128]
            mo_ref[slot] = rmax(val, None)

        def rmax(st, m8):
            cm = jnp.max(st.reshape(st.shape[0] // 8, 8, TQ), axis=0)
            return cm if m8 is None else jnp.maximum(m8, cm)

        def p_store(r0, r1, e):
            p_ref[r0 // 2:r1 // 2, :] = pltpu.bitcast(jnp.exp2(e).astype(bf16), u32)

        def pv_unit(i, u, acc):
            ks = slice(u * KC, (u + 1) * KC)
            p = pltpu.bitcast(p_ref[u * KC // 2:(u + 1) * KC // 2, :], bf16)
            pv = jnp.dot(pltpu.bitcast(vt_ref[item(i)[0], :, ks], bf16), p, preferred_element_type=f32)
            return pv if acc is None else acc + pv

        def finish(i, acc, chk):
            hc, _, _, qc = item(i)
            ot_ref[hc, :, dsl(qc, TQ, TQ)] = acc
            ok = jnp.where(jnp.abs(acc) < BIG, 0.0, 1.0)
            return jnp.maximum(chk, jnp.max(ok.reshape(4, 8, TQ), axis=0))

        def shift_of(slot):
            return -(jnp.max(mo_ref[slot], axis=0, keepdims=True).astype(bf16).astype(f32))

        def vpu_chain(h, q0, kg, t, slot):
            qi = (q0 // 128 + t) * H + h
            qb = jnp.concatenate([qf_ref[qi, pl.ds(d, 8, stride=0), :] for d in range(DH)], axis=0)
            pr = (kb_ref[h % NKB, kg] * qb).reshape(DH // 2, 16, 128)
            s2 = jnp.sum(pr, axis=0)
            res = s2[0:8] + s2[8:16]
            so_ref[slot * NTL + t, kg * 8:(kg + 1) * 8, :] = res
            return res

        def stage(i, s, acc, chk, first=False, extra=None, tie_qk=None):
            g = item(i)[1]
            cneg = shift_of(s)
            qm = make_qm(i, cneg)
            for c in range(NC):
                if c < LAG:
                    if not first:
                        acc = pv_unit(i - 1, NC - LAG + c, acc)
                        if c == LAG - 1:
                            chk = finish(i - 1, acc, chk)
                            acc = None
                else:
                    acc = pv_unit(i, c - LAG, acc)
                r0, r1 = c * KC, (c + 1) * KC
                st = qk_rows(g, qm, r0 + OFFR[c], r1)
                if tie_qk is not None:
                    st = tie_qk(st, s * NC + c)
                if OFFR[c]:
                    st = jnp.concatenate([so_load(s, OFFS[c], OFFS[c + 1]) + cneg, st], axis=0)
                p_store(r0, r1, st)
                if extra is not None:
                    extra(c)
            return acc, chk

        kps = gather_keys(NA - 1, OFFR[12:16])
        for i_ in range(AHEAD + 1):
            so_store((i_ - 1) % NS, jnp.dot(pltpu.bitcast(ko_ref[0], bf16), make_qm(i_, None),
                                            preferred_element_type=f32))
        proj((NA - 1) * TA, xnt_load(), 2, 3)
        zpad4 = jnp.zeros((32 - DH, D), f32)
        wof = wo_ref[...].astype(f32)
        wop = jnp.concatenate(
            [blk for h in range(H) for blk in (wof[h * DH:(h + 1) * DH, :], zpad4)], axis=0)
        wot_ref[...] = pltpu.bitcast(wop.astype(bf16).T, u32)
        prebuild(NA - 1, kps)
        carry0 = stage(0, NS - 1, None, jnp.zeros((8, TQ), f32), first=True)

        pltpu.make_async_copy(wf_ref, wf_ref, sems.at[6]).wait()

        def split_tie(y, ties):
            R, C = y.shape[0] // 8, y.shape[1] // 128
            newv = {}
            for (r, c), fn_ in ties.items():
                newv[(r, c)] = fn_(y[r * 8:(r + 1) * 8, c * 128:(c + 1) * 128])
            cols = []
            for c in range(C):
                rows = sorted(r for (r, c_) in newv if c_ == c)
                pieces, lo = [], 0
                for r in rows:
                    if r > lo:
                        pieces.append(y[lo * 8:r * 8, c * 128:(c + 1) * 128])
                    pieces.append(newv[(r, c)])
                    lo = r + 1
                if lo < R:
                    pieces.append(y[lo * 8:R * 8, c * 128:(c + 1) * 128])
                cols.append(pieces[0] if len(pieces) == 1 else jnp.concatenate(pieces, axis=0))
            return jnp.concatenate(cols, axis=1)

        def pos_of(i_, R, pair):
            if pair:
                return (i_ % (2 * R)) // 2, 2 * (i_ // (2 * R)) + i_ % 2
            return i_ % R, i_ // R

        def att_body(t, carry):
            hstate = {}
            never = lax.broadcasted_iota(jnp.int32, (8, 128), 0) < jnp.minimum(t, 0)
            ninf = jnp.where(never, 0.0, -jnp.inf)

            def tied(v, res):
                if SELTIE == 1:
                    return jnp.where(never, res, v)
                return v + (res - res)
            jobs = []
            for s in range(NS):
                hh, _, _, q0 = item(jnp.minimum(t * NS + s + AHEAD + 1, NI - 1))
                for kb_ in range(NKG):
                    for tt in range(NTL):
                        kg = (kb_ // NTL) * NTL + (kb_ + tt) % NTL if (LATIN and kb_ < (NKG // NTL) * NTL) else kb_
                        jobs.append((hh, q0, kg, tt, (s + AHEAD) % NS))
            trs = {n: (TR2 if (TR2 and n % TR2E == 0) else TR) for n in range(ALAST + 1)}
            for b_ in range(NB - 1):
                for o_ in LOWO:
                    trs[FPOS[b_] + o_] = TRL
            n_ffn = max(len(jobs) - sum(len(v) for v in trs.values()), 0)
            total = (NB - 1) * (WG + WU + WD) + (0 if BG else WG)
            st_ = {"time": 0, "fdone": 0, "done": 0, "step": 0}
            bst = {"n": 0}
            mx = [None] * NTL

            def chain_tie(v):
                if st_["done"] >= len(jobs):
                    return v
                job = jobs[st_["done"]]
                s_job = st_["done"] // (NKG * NTL)
                assert (s_job + AHEAD - NS + 1) * NC <= st_["step"] < (s_job + AHEAD) * NC, (s_job, st_)
                k_in = (st_["done"] % (NKG * NTL)) // NTL
                st_["done"] += 1
                res = vpu_chain(*job)
                tt = job[3]
                mx[tt] = res if k_in == 0 else jnp.maximum(mx[tt], res)
                if k_in == NKG - 1:
                    mo_ref[job[4], :, tt * 128:(tt + 1) * 128] = mx[tt]
                return tied(v, mx[tt])

            def tie(y, w, pair=False, skip=0):
                st_["time"] += w
                want = (n_ffn * st_["time"]) // total
                n = want - st_["fdone"]
                st_["fdone"] = want
                if n == 0:
                    return y
                R, C = y.shape[0] // 8, y.shape[1] // 128
                lo = (R * C * skip) // 100
                idx = [lo + ((k + 1) * (R * C - lo)) // n - 1 for k in range(n)]
                return split_tie(y, {pos_of(i_, R, pair): chain_tie for i_ in idx})

            def tie_qk(st, n):
                st_["step"] = n
                if n == ALAST:
                    bst["rel"] = st[0:8, 0:128]
                if n in trs:
                    return split_tie(st, {(st.shape[0] // 8 - r, k % NTL): chain_tie for k, r in enumerate(trs[n])})
                return st

            def build_tie(v):
                k_, d = divmod(bst["n"], DH)
                bst["n"] += 1
                hb = 5 + 2 * t + k_
                if d == 0:
                    hc_ = jnp.minimum(hb, H - 1)
                    bst["kf"] = head_k(ko_ref[hc_ // 4], hc_, bst["rel"])
                res = build_col(bst["kf"], hb % NKB, slice(None), d)
                v = v + (res - res)
                if d == DH - RELB:
                    bst["rel"] = v
                return v

            def tie_build(y, ncols, skip, pair=False):
                R, C = y.shape[0] // 8, y.shape[1] // 128
                lo = (R * C * skip) // 100
                idx = [lo + ((n + 1) * (R * C - lo)) // ncols - 1 for n in range(ncols)]
                return split_tie(y, {pos_of(i_, R, pair): build_tie for i_ in idx})

            def ffn_up(b):
                last = b == NB - 1
                xq = pltpu.bitcast(xn_ref[b * TF // 2:(b + 1) * TF // 2, :], bf16)
                gt = jnp.dot(xq, wf_ref[0, t], preferred_element_type=f32)
                gt = tie_build(gt, BC[0], BSKIP) if (last and BG) else tie(gt, WG)
                if last and not BG:
                    bst["rel"] = gt[TF - 8:TF, FC - 128:FC]
                up = jnp.dot(xq, wf_ref[1, t], preferred_element_type=f32)
                up = tie_build(up, BC[1], 0 if BG else BSKIP) if last else tie(up, WU)
                gh = 0.5 * gt
                hstate[b] = ((gh * up) * (jnp.tanh(gh) + 1.0)).astype(bf16)

            def ffn_down(b):
                tsl = slice(b * TF, (b + 1) * TF)
                dn = lax.dot_general(wf_ref[2, t], hstate.pop(b), NT, preferred_element_type=f32)
                acc_ref[:, tsl] += tie_build(dn, BC[2], 0, True) if b == NB - 1 else tie(dn, WD, True, DSKIP)

            sched = {}
            for b in range(NB):
                sched[FPOS[b]] = functools.partial(ffn_up, b)
                sched[FPOS[b] + FPD] = functools.partial(ffn_down, b)

            for s in range(NS):
                def extra(c, s=s):
                    fn_ = sched.get(s * NC + c)
                    if fn_ is not None:
                        fn_()
                carry = stage(t * NS + s + 1, s, *carry, extra=extra, tie_qk=tie_qk)
            assert st_["done"] == len(jobs) and bst["n"] == 2 * DH, (st_, len(jobs), bst["n"])
            return carry

        acc, chk = lax.fori_loop(0, NIT, att_body, carry0)

        state = {"n": 0, "lo": 0}
        RH = D // RS

        def normalized(sl):
            a = ot_ref[:, :, sl]
            l = a[:, DH:DH + 1, :]
            r0 = pl.reciprocal(l, approx=True)
            r0 = r0 * (2.0 - l * r0)
            return (a * r0).reshape(H * 32, OW).astype(bf16)

        def next_piece():
            b, r = divmod(state["n"], RS)
            sl = slice(b * OW, (b + 1) * OW)
            rs = slice(r * RH, (r + 1) * RH)
            if r == 0:
                state["o"] = normalized(sl)
            wo_t = pltpu.bitcast(wot_ref[r * RH // 2:(r + 1) * RH // 2, :], bf16)
            o = (xt_ref[rs, sl].astype(f32) + acc_ref[rs, sl]) + jnp.dot(wo_t, state["o"], preferred_element_type=f32)
            outb_ref[rs, sl] = o.astype(bf16)
            state["n"] += 1
            if r == RS - 1 and ((b + 1) % OG == 0 or b + 1 >= NO - 1):
                c0_, c1_ = state["lo"] * OW, (b + 1) * OW
                pltpu.make_async_copy(outb_ref.at[:, c0_:c1_], out_hbm.at[:, c0_:c1_], osem.at[0]).start()
                state["lo"] = b + 1

        for c in range(LAG):
            acc = pv_unit(NI - 1, NC - LAG + c, acc)
            next_piece()
        chk = finish(NI - 1, acc, chk)
        while state["n"] < NO * RS:
            next_piece()
        bad = jnp.max(chk)
        pltpu.make_async_copy(outb_ref, out_hbm, osem.at[0]).wait()

        if FALLBACK:
            @pl.when((bad > 0.0) if not FORCE else (bad >= 0.0))
            def _():
                def fb_item(i, carry):
                    h, g, _, q0 = item(i)
                    qm = make_qm(i, None)

                    def qk(c, m8):
                        kk = pltpu.bitcast(k_ref[g, dsl(c * (KC // 2), KC // 2, KC // 2), :], bf16)
                        st = jnp.dot(kk, qm, preferred_element_type=f32)
                        s_ref[dsl(c * KC, KC, KC), :] = st
                        return rmax(st, m8)
                    m8 = lax.fori_loop(0, NC, qk, jnp.full((8, TQ), -jnp.inf, f32))
                    m = jnp.max(m8, axis=0, keepdims=True)

                    def pv(c, a):
                        p = jnp.exp2(s_ref[dsl(c * KC, KC, KC), :] - m).astype(bf16)
                        vv = pltpu.bitcast(vt_ref[h, :, dsl(c * KC, KC, KC)], bf16)
                        return a + jnp.dot(vv, p, preferred_element_type=f32)
                    ot_ref[h, :, dsl(q0, TQ, TQ)] = lax.fori_loop(0, NC, pv, jnp.zeros((32, TQ), f32))
                    return carry
                lax.fori_loop(0, NI, fb_item, 0)

                def fb_out(b, carry):
                    sl = dsl(b * OW, OW, OW)
                    o = (xt_ref[:, sl].astype(f32) + acc_ref[:, sl]) + jnp.dot(
                        pltpu.bitcast(wot_ref[...], bf16), normalized(sl), preferred_element_type=f32)
                    outb_ref[:, sl] = o.astype(bf16)
                    return carry
                lax.fori_loop(0, NO, fb_out, 0)
                cp = pltpu.make_async_copy(outb_ref, out_hbm, osem.at[0])
                cp.start()
                cp.wait()

    @jax.jit
    def fn(A_x, A_wqkv, A_wo, B_x, B_w1, B_w3, B_w2):
        xt = A_x.reshape(S, D).T
        w2t = B_w2.T
        anyspec = pl.BlockSpec(memory_space=pl.ANY)
        out = pl.pallas_call(
            kernel,
            in_specs=[anyspec] * 6,
            out_specs=anyspec,
            out_shape=jax.ShapeDtypeStruct((D, S), bf16),
            scratch_shapes=[
                pltpu.VMEM((D, S), bf16), pltpu.VMEM((D, 3 * D), bf16), pltpu.VMEM((D, D), bf16),
                pltpu.VMEM((3, NIT, D, FC), bf16), pltpu.VMEM((D, S), bf16),
                pltpu.VMEM((3 * HD, D), u32), pltpu.VMEM((HD, 512), u32),
                pltpu.VMEM((S // 2, D), u32), pltpu.VMEM((HD, TA), u32), pltpu.VMEM((HD, SPLIT0), u32),
                pltpu.VMEM((NG, GW // 2, S), u32), pltpu.VMEM((NG, S // 2, 128), u32),
                pltpu.VMEM((H, 16, S), u32), pltpu.VMEM((H, 32, S), f32), pltpu.VMEM((D, S), f32),
                pltpu.VMEM(((S // 128) * H, 32, 128), f32), pltpu.VMEM((NS * NTL, NOFF, 128), f32), pltpu.VMEM((NS, 8, TQ), f32),
                pltpu.VMEM((NKB, NKG, DH * 8, 128), f32), pltpu.VMEM((NG, NOFF // 2, 128), u32),
                pltpu.VMEM((S // 2, TQ), u32), pltpu.VMEM((S, TQ), f32),
                pltpu.SemaphoreType.DMA((7,)), pltpu.SemaphoreType.DMA((1,))],
            compiler_params=pltpu.CompilerParams(vmem_limit_bytes=110 * 1024 * 1024),
            name="fusedk",
        )(xt, A_wqkv, A_wo, B_w1, B_w3, w2t)
        return out.T.reshape(1, S, D)
    return fn


_impl = build(NOFF=240)


@jax.jit
def pallas_parallel_sum__softmax_full_mha__glu_gated_swiglu__prompt_kernel(
    A_x: jax.Array,
    A_wqkv: jax.Array,
    A_wo: jax.Array,
    B_x: jax.Array,
    B_w1: jax.Array,
    B_w3: jax.Array,
    B_w2: jax.Array,
):
    return _impl(A_x, A_wqkv, A_wo, B_x, B_w1, B_w3, B_w2)
```

```python
import functools
import math

import jax
import jax.numpy as jnp
from jax import lax
from jax.experimental import pallas as pl
from jax.experimental.pallas import tpu as pltpu

S, D, H, DH, F = 2048, 448, 16, 28, 1792
NG, GW, HD = 4, 112, 224
EPS = 1e-5
QSCALE = (DH ** -0.5) * math.log2(math.e)
NT = (((1,), (1,)), ((), ()))
f32, bf16, u32 = jnp.float32, jnp.bfloat16, jnp.uint32
BIG, SMALL = 2.0 ** 60, 2.0 ** -60


def _build():
    NOFF, OA = 240, 64
    TR = (13, 10, 7, 4, 1)
    FB, FPOS, FPD = (12, 4), (40, 138), 4
    WG, WU, WD = 1100, 950, 900
    BC, BSKIP, RELB = (20, 24, 12), 20, 8
    QB0, QBE = 4, 6
    TQ = TA = 512
    KC, FC, OW, OG, RS, SPLIT0 = 128, 256, 128, 2, 2, 384
    NS, LAG, AHEAD, NKB = 9, 3, 3, 8
    NQ, NC, NA, NO, NTL = S // TQ, S // KC, S // TA, S // OW, TQ // 128
    NI = NQ * H
    NIT = (NI - 1) // NS
    NKG = NOFF // 8
    NJ = NKG * NTL
    ALAST = FPOS[-1]
    assert NOFF % 16 == 0 and F // FC == NIT and sum(FB) == S // 128 and sum(BC) == 2 * DH

    def _pat(n):
        return [16 * (((c_ + 1) * (n // 16)) // 4 - (c_ * (n // 16)) // 4) for c_ in range(4)]
    OFFR = _pat(OA) * 3 + _pat(NOFF - 3 * OA)
    OFFS = [sum(OFFR[:c_]) for c_ in range(NC + 1)]
    assert OFFS[NC] == NOFF

    def kernel(xt_hbm, wqkv_hbm, wo_hbm, w1_hbm, w3_hbm, w2t_hbm, out_hbm,
               xt_ref, wqkv_ref, wo_ref, wf_ref, outb_ref,
               wt_ref, wot_ref, xn_ref, xnt_ref, kt0_ref, qt_ref, k_ref, vt_ref, ot_ref, acc_ref,
               qf_ref, qb_ref, so_ref, mo_ref, vm_ref, kb_ref, ko_ref, p_ref, s_ref, sems, osem):

        def wcopy(c0, c1, k):
            return pltpu.make_async_copy(wqkv_hbm.at[:, c0:c1], wqkv_ref.at[:, c0:c1], sems.at[k])

        cp_x = [pltpu.make_async_copy(xt_hbm.at[:, c * TA:(c + 1) * TA], xt_ref.at[c], sems.at[c])
                for c in range(NA)]
        cp_wk, cp_wq, cp_wv = wcopy(384, 896, 4), wcopy(0, 384, 5), wcopy(896, 3 * D, 6)
        cp_wo = pltpu.make_async_copy(wo_hbm, wo_ref, sems.at[7])
        for cp in [cp_x[0], cp_wk, cp_wq, cp_wv] + cp_x[1:] + [cp_wo]:
            cp.start()
        acc_ref[...] = jnp.zeros((D, S), f32)
        cp_x[0].wait()
        for k, src in enumerate((w1_hbm, w3_hbm, w2t_hbm)):
            for j in range(NIT):
                pltpu.make_async_copy(src.at[:, j * FC:(j + 1) * FC], wf_ref.at[k, j], sems.at[8]).start()

        def dsl(start, size, align):
            return pl.ds(start, size) if isinstance(start, int) else pl.ds(pl.multiple_of(start, align), size)

        def first_row(n_rows, n, dtype):
            return jnp.where(lax.broadcasted_iota(jnp.int32, (n_rows, n), 0) == 0, 1.0, 0.0).astype(dtype)

        def layernorm(c):
            xt = xt_ref[c].astype(f32)
            mu = jnp.sum(xt, axis=0, keepdims=True) * (1.0 / D)
            xc = xt - mu
            var = jnp.sum(xc * xc, axis=0, keepdims=True) * (1.0 / D)
            return (xc * lax.rsqrt(var + EPS)).astype(bf16)

        def pack_k(kt):
            n = kt.shape[1]
            return pltpu.bitcast(jnp.concatenate([kt, first_row(128 - GW, n, bf16)], axis=0).T, u32)

        def proj(t0, xnt, p0, p1):
            n = xnt.shape[1]
            sl = dsl(t0, n, TA)
            yy = jnp.dot(pltpu.bitcast(wt_ref[p0 * HD:p1 * HD, :], bf16), xnt, preferred_element_type=f32)
            for part in range(p0, p1):
                y = yy[(part - p0) * D:(part - p0 + 1) * D, :]
                if part == 0:
                    yk = y.astype(bf16)
                    for g in range(NG):
                        k_ref[g, dsl(t0 // 2, n // 2, TA // 2), :] = pack_k(yk[GW * g:GW * (g + 1), :])
                elif part == 1:
                    yq = (y * QSCALE).astype(bf16)
                    yf = yq.astype(f32)
                    for h in range(H):
                        yh = jnp.concatenate([yf[h * DH:(h + 1) * DH, :], jnp.zeros((32 - DH, n), f32)], axis=0)
                        for t in range(n // 128):
                            qf_ref[(t0 // 128 + t) * H + h] = yh[:, t * 128:(t + 1) * 128]
                    for g in range(NG):
                        qt_ref[g, :, sl] = pltpu.bitcast(yq[GW * g:GW * (g + 1), :], u32)
                else:
                    vm_ref[dsl((t0 // TA) * 8, 8, 8), :] = jnp.max(
                        jnp.abs(y).reshape(D // 8, 8, n), axis=0)
                    vpad = first_row(32 - DH, n, f32)
                    for h in range(H):
                        vt_ref[h, :, sl] = pltpu.bitcast(
                            jnp.concatenate([y[DH * h:DH * (h + 1), :], vpad], axis=0).astype(bf16), u32)

        def head_k(kp, h, rel=None):
            if rel is not None:
                z = pltpu.bitcast(rel - rel, u32)
                kp = kp | jnp.concatenate([z] * (kp.shape[0] // 8), axis=0)
            kp = pltpu.roll(kp, (128 - DH * (h % 4)) % 128, 1)
            return pltpu.bitcast(kp, bf16).astype(f32)

        def build_col(kf, slot, kgs, d):
            n = kf.shape[0]
            bc = jnp.broadcast_to(kf[:, d:d + 1], (n, 128))
            kb_ref[slot, kgs, d * 8:(d + 1) * 8, :] = bc.reshape(n // 8, 8, 128)
            return bc[n - 8:n, :]

        def gather_keys(c, pat):
            n = sum(pat)
            out = []
            for g in range(NG):
                kp = jnp.concatenate([k_ref[g, dsl(c * (TA // 2) + j * 64, r // 2, 64), :]
                                      for j, r in enumerate(pat) if r], axis=0)
                ko_ref[g, dsl(c * (OA // 2), n // 2, 8), :] = kp
                out.append(kp)
            return out

        def prebuild(c, kps):
            n = 2 * kps[0].shape[0]
            for h in range(1, 5):
                kf = head_k(kps[h // 4], h)
                for d in range(DH):
                    build_col(kf, h, pl.ds(c * (OA // 8), n // 8), d)

        def xnt_load(c0=0, c1=TA):
            return pltpu.bitcast(xnt_ref[:, c0:c1], bf16)

        xnt_ref[...] = pltpu.bitcast(layernorm(0), u32)
        cp_wk.wait()
        wt_ref[0:HD, :] = pltpu.bitcast(wqkv_ref[:, 384:896].T[64:512, :], u32)
        kt0_ref[...] = pltpu.bitcast(jnp.dot(pltpu.bitcast(wt_ref[0:HD, :], bf16), xnt_load(0, SPLIT0),
                                             preferred_element_type=f32).astype(bf16), u32)
        xn_ref[0:TA // 2, :] = pltpu.bitcast(xnt_load().T, u32)
        cp_wq.wait()
        cp_wv.wait()
        proj(SPLIT0, xnt_load(SPLIT0, TA), 0, 1)
        for g in range(NG):
            k_ref[g, 0:SPLIT0 // 2, :] = pack_k(pltpu.bitcast(kt0_ref[GW // 2 * g:GW // 2 * (g + 1), :], bf16))
        wt_ref[HD:2 * HD, :] = pltpu.bitcast(wqkv_ref[:, 0:512].T[0:D, :], u32)
        wt_ref[2 * HD:3 * HD, :] = pltpu.bitcast(wqkv_ref[:, 896:3 * D].T, u32)
        proj(0, xnt_load(), 1, 2)
        for cp in cp_x[1:]:
            cp.wait()

        def a_body(c, carry):
            kps = gather_keys(c - 1, OFFR[0:4])
            proj((c - 1) * TA, xnt_load(), 2, 3)
            xnt = layernorm(c)
            xn_ref[dsl(c * (TA // 2), TA // 2, TA // 2), :] = pltpu.bitcast(xnt.T, u32)
            proj(c * TA, xnt, 0, 2)
            xnt_ref[...] = pltpu.bitcast(xnt, u32)
            prebuild(c - 1, kps)
            return carry
        lax.fori_loop(1, NA, a_body, 0)
        cp_wo.wait()

        rowq = lax.broadcasted_iota(jnp.int32, (GW // 2, TQ), 0)
        row16 = lax.broadcasted_iota(jnp.int32, (128 - GW, TQ), 0)

        def item(i):
            h = i // NQ
            return h, h // 4, h % 4, (i % NQ) * TQ

        def make_qm(i, cneg):
            _, g, j, q0 = item(i)
            lo = j * (DH // 2)
            qm = jnp.where((rowq >= lo) & (rowq < lo + DH // 2), qt_ref[g, :, dsl(q0, TQ, TQ)], jnp.uint32(0))
            if cneg is None:
                tail = jnp.zeros((64 - GW // 2, TQ), u32)
            else:
                tail = pltpu.bitcast(jnp.where(row16 == 0, cneg, 0.0).astype(bf16), u32)
            return pltpu.bitcast(jnp.concatenate([qm, tail], axis=0), bf16)

        def rmax(st, m8):
            cm = jnp.max(st.reshape(st.shape[0] // 8, 8, TQ), axis=0)
            return cm if m8 is None else jnp.maximum(m8, cm)

        def pv_unit(i, u, acc):
            p = pltpu.bitcast(p_ref[u * KC // 2:(u + 1) * KC // 2, :], bf16)
            vt = pltpu.bitcast(vt_ref[item(i)[0], :, u * KC:(u + 1) * KC], bf16)
            pv = jnp.dot(vt, p, preferred_element_type=f32)
            return pv if acc is None else acc + pv

        def finish(i, acc, chk):
            h, _, _, q0 = item(i)
            ot_ref[h, :, dsl(q0, TQ, TQ)] = acc
            return jnp.maximum(chk[0], acc[24:32, :]), jnp.minimum(chk[1], acc[24:32, :])

        def build_qb(i, k, n, z):
            h, _, _, q0 = item(i)
            t, gq = divmod(n, 4)
            nr = min(8, DH - gq * 8)
            q = qf_ref[(q0 // 128 + t) * H + h, gq * 8:(gq + 1) * 8, :] + z
            qb_ref[k * NTL + t, gq * 64:gq * 64 + nr * 8, :] = jnp.concatenate(
                [jnp.broadcast_to(q[d:d + 1, :], (8, 128)) for d in range(nr)], axis=0)

        def stage(i, s, acc, chk, hook, first=False, extra=None):
            g = item(i)[1]
            cneg = -(jnp.max(mo_ref[s], axis=0, keepdims=True).astype(bf16).astype(f32))
            qm = make_qm(i, cneg)
            for c in range(NC):
                if c >= LAG:
                    acc = pv_unit(i, c - LAG, acc)
                elif not first:
                    acc = pv_unit(i - 1, NC - LAG + c, acc)
                    if c == LAG - 1:
                        chk = finish(i - 1, acc, chk)
                        acc = None
                r0, r1 = c * KC + OFFR[c], (c + 1) * KC
                st = jnp.dot(pltpu.bitcast(k_ref[g, r0 // 2:r1 // 2, :], bf16), qm, preferred_element_type=f32)
                st = hook(st, s * NC + c)
                if OFFR[c]:
                    so = jnp.concatenate([so_ref[s * NTL + t, OFFS[c]:OFFS[c + 1], :] for t in range(NTL)], axis=1)
                    st = jnp.concatenate([so + cneg, st], axis=0)
                p_ref[c * KC // 2:(c + 1) * KC // 2, :] = pltpu.bitcast(jnp.exp2(st).astype(bf16), u32)
                if extra is not None:
                    extra(s * NC + c)
            return acc, chk

        kps = gather_keys(NA - 1, OFFR[12:16])
        for i_ in range(AHEAD + 1):
            val = jnp.dot(pltpu.bitcast(ko_ref[0], bf16), make_qm(i_, None), preferred_element_type=f32)
            for t in range(NTL):
                so_ref[((i_ - 1) % NS) * NTL + t] = val[:, t * 128:(t + 1) * 128]
            mo_ref[(i_ - 1) % NS] = rmax(val, None)
        proj((NA - 1) * TA, xnt_load(), 2, 3)
        zpad4 = jnp.zeros((32 - DH, D), f32)
        wof = wo_ref[...].astype(f32)
        wop = jnp.concatenate(
            [blk for h in range(H) for blk in (wof[h * DH:(h + 1) * DH, :], zpad4)], axis=0)
        wot_ref[...] = pltpu.bitcast(wop.astype(bf16).T, u32)
        prebuild(NA - 1, kps)

        def hook0(st, n):
            for k in range(NS):
                v = st[(k + 2) * 8:(k + 3) * 8, 0:128]
                build_qb(k + AHEAD + 1, k, n % NC, v - v)
            return st
        one = jnp.ones((8, TQ), f32)
        carry0 = stage(0, NS - 1, None, (one, one), hook0, first=True)

        pltpu.make_async_copy(wf_ref, wf_ref, sems.at[8]).wait()

        def split_tie(y, pos, fn):
            R, C = y.shape[0] // 8, y.shape[1] // 128
            newv = {(r, c): fn(y[r * 8:(r + 1) * 8, c * 128:(c + 1) * 128]) for (r, c) in pos}
            cols = []
            for c in range(C):
                pieces, lo = [], 0
                for r in sorted(r for (r, c_) in newv if c_ == c):
                    if r > lo:
                        pieces.append(y[lo * 8:r * 8, c * 128:(c + 1) * 128])
                    pieces.append(newv[(r, c)])
                    lo = r + 1
                if lo < R:
                    pieces.append(y[lo * 8:R * 8, c * 128:(c + 1) * 128])
                cols.append(pieces[0] if len(pieces) == 1 else jnp.concatenate(pieces, axis=0))
            return jnp.concatenate(cols, axis=1)

        def spread(y, n, skip, pair):
            R, C = y.shape[0] // 8, y.shape[1] // 128
            lo = (R * C * skip) // 100
            idx = [lo + ((k + 1) * (R * C - lo)) // n - 1 for k in range(n)]
            if pair:
                return [((i_ % (2 * R)) // 2, 2 * (i_ // (2 * R)) + i_ % 2) for i_ in idx]
            return [(i_ % R, i_ // R) for i_ in idx]

        def att_body(t, carry):
            heads = [item(jnp.minimum(t * NS + k + AHEAD + 1, NI - 1))[0] for k in range(NS)]
            n_ffn = NS * NJ - (ALAST + 1) * len(TR)
            total = sum(FB[:-1]) * (WG + WU + WD)
            st_ = {"time": 0, "fdone": 0, "done": 0, "step": 0, "nb": 0}
            mx = [None] * NTL
            hstate = {}

            def qb_next(k, n, z):
                build_qb(jnp.minimum((t + 1) * NS + k + AHEAD + 1, NI - 1), k, n, z)

            def chain_tie(v):
                k, n_in = divmod(st_["done"], NJ)
                kg, tt = divmod(n_in, NTL)
                slot = (k + AHEAD) % NS
                assert (k + AHEAD - NS + 1) * NC <= st_["step"] < (k + AHEAD) * NC
                st_["done"] += 1
                pr = (kb_ref[heads[k] % NKB, kg] * qb_ref[k * NTL + tt]).reshape(DH // 2, 16, 128)
                s2 = jnp.sum(pr, axis=0)
                res = s2[0:8] + s2[8:16]
                so_ref[slot * NTL + tt, kg * 8:(kg + 1) * 8, :] = res
                mx[tt] = res if kg == 0 else jnp.maximum(mx[tt], res)
                if kg == NKG - 1:
                    mo_ref[slot, :, tt * 128:(tt + 1) * 128] = mx[tt]
                z = mx[tt] - mx[tt]
                nq = n_in - QB0
                if k > 0 and nq >= 0 and nq % QBE == 0 and nq // QBE < 16:
                    qb_next(k - 1, nq // QBE, z)
                return v + z

            def build_tie(v):
                k_, d = divmod(st_["nb"], DH)
                st_["nb"] += 1
                hb = 5 + 2 * t + k_
                if d == 0:
                    hc = jnp.minimum(hb, H - 1)
                    st_["kf"] = head_k(ko_ref[hc // 4], hc, st_["rel"])
                res = build_col(st_["kf"], hb % NKB, slice(None), d)
                z = res - res
                v = v + z
                if st_["nb"] % 3 == 0 and st_["nb"] // 3 <= 16:
                    qb_next(NS - 1, st_["nb"] // 3 - 1, z)
                if d == DH - RELB:
                    st_["rel"] = v
                return v

            def tie(y, b, w, kind):
                pair = kind == 2
                if b == len(FB) - 1:
                    return split_tie(y, spread(y, BC[kind], BSKIP if kind == 0 else 0, pair), build_tie)
                st_["time"] += w * FB[b]
                n = (n_ffn * st_["time"]) // total - st_["fdone"]
                st_["fdone"] += n
                return split_tie(y, spread(y, n, 0, pair), chain_tie)

            def hook(st, n):
                st_["step"] = n
                if n == ALAST:
                    st_["rel"] = st[0:8, 0:128]
                if n > ALAST:
                    return st
                return split_tie(st, [(st.shape[0] // 8 - r, k % NTL) for k, r in enumerate(TR)], chain_tie)

            def ffn_up(b):
                t0, t1 = sum(FB[:b]) * 128, sum(FB[:b + 1]) * 128
                xq = pltpu.bitcast(xn_ref[t0 // 2:t1 // 2, :], bf16)
                gt = tie(jnp.dot(xq, wf_ref[0, t], preferred_element_type=f32), b, WG, 0)
                up = tie(jnp.dot(xq, wf_ref[1, t], preferred_element_type=f32), b, WU, 1)
                gh = 0.5 * gt
                hstate[b] = ((gh * up) * (jnp.tanh(gh) + 1.0)).astype(bf16)

            def ffn_down(b):
                t0, t1 = sum(FB[:b]) * 128, sum(FB[:b + 1]) * 128
                dn = lax.dot_general(wf_ref[2, t], hstate.pop(b), NT, preferred_element_type=f32)
                acc_ref[:, t0:t1] += tie(dn, b, WD, 2)

            sched = {}
            for b in range(len(FB)):
                sched[FPOS[b]] = functools.partial(ffn_up, b)
                sched[FPOS[b] + FPD] = functools.partial(ffn_down, b)

            def extra(n):
                if n in sched:
                    sched[n]()

            for s in range(NS):
                carry = stage(t * NS + s + 1, s, *carry, hook, extra=extra)
            assert st_["done"] == NS * NJ and st_["nb"] == 2 * DH
            return carry

        acc, chk = lax.fori_loop(0, NIT, att_body, carry0)

        RH, PB = D // RS, TA // OW
        state = {"n": 0, "lo": 0}

        def normalized(sl):
            a = ot_ref[:, :, sl]
            l = a[:, DH:DH + 1, :]
            r0 = pl.reciprocal(l, approx=True)
            r0 = r0 * (2.0 - l * r0)
            return (a * r0).reshape(H * 32, OW).astype(bf16)

        def next_piece():
            b, r = divmod(state["n"], RS)
            sl = slice(b * OW, (b + 1) * OW)
            rs = slice(r * RH, (r + 1) * RH)
            if r == 0:
                state["o"] = normalized(sl)
            wo_t = pltpu.bitcast(wot_ref[r * RH // 2:(r + 1) * RH // 2, :], bf16)
            x = xt_ref[b // PB, rs, (b % PB) * OW:(b % PB + 1) * OW].astype(f32)
            o = (x + acc_ref[rs, sl]) + jnp.dot(wo_t, state["o"], preferred_element_type=f32)
            outb_ref[rs, sl] = o.astype(bf16)
            state["n"] += 1
            if r == RS - 1 and ((b + 1) % OG == 0 or b + 1 >= NO - 1):
                c0, c1 = state["lo"] * OW, (b + 1) * OW
                pltpu.make_async_copy(outb_ref.at[:, c0:c1], out_hbm.at[:, c0:c1], osem.at[0]).start()
                state["lo"] = b + 1

        for c in range(LAG):
            acc = pv_unit(NI - 1, NC - LAG + c, acc)
            next_piece()
        chk = finish(NI - 1, acc, chk)
        while state["n"] < NO * RS:
            next_piece()
        lhi, llo = chk[0][DH - 24:DH - 23, :], chk[1][DH - 24:DH - 23, :]
        ok = (lhi < BIG) & (llo > SMALL) & (jnp.max(vm_ref[...], axis=0, keepdims=True) < BIG)
        bad = jnp.max(jnp.where(ok, 0.0, 1.0))
        pltpu.make_async_copy(outb_ref, out_hbm, osem.at[0]).wait()

        @pl.when(bad > 0.0)
        def _():
            def fb_item(i, carry):
                h, g, _, q0 = item(i)
                qm = make_qm(i, None)

                def qk(c, m8):
                    kk = pltpu.bitcast(k_ref[g, dsl(c * (KC // 2), KC // 2, KC // 2), :], bf16)
                    st = jnp.dot(kk, qm, preferred_element_type=f32)
                    s_ref[dsl(c * KC, KC, KC), :] = st
                    return rmax(st, m8)
                m8 = lax.fori_loop(0, NC, qk, jnp.full((8, TQ), -jnp.inf, f32))
                m = jnp.max(m8, axis=0, keepdims=True)

                def pv(c, a):
                    p = jnp.exp2(s_ref[dsl(c * KC, KC, KC), :] - m).astype(bf16)
                    vt = pltpu.bitcast(vt_ref[h, :, dsl(c * KC, KC, KC)], bf16)
                    return a + jnp.dot(vt, p, preferred_element_type=f32)
                ot_ref[h, :, dsl(q0, TQ, TQ)] = lax.fori_loop(0, NC, pv, jnp.zeros((32, TQ), f32))
                return carry
            lax.fori_loop(0, NI, fb_item, 0)

            def fb_out(b, carry):
                sl = dsl(b * OW, OW, OW)
                x = xt_ref[b // PB, :, dsl((b % PB) * OW, OW, OW)].astype(f32)
                o = (x + acc_ref[:, sl]) + jnp.dot(
                    pltpu.bitcast(wot_ref[...], bf16), normalized(sl), preferred_element_type=f32)
                outb_ref[:, sl] = o.astype(bf16)
                return carry
            lax.fori_loop(0, NO, fb_out, 0)
            cp = pltpu.make_async_copy(outb_ref, out_hbm, osem.at[0])
            cp.start()
            cp.wait()

    scratch = [
        pltpu.VMEM((NA, D, TA), bf16), pltpu.VMEM((D, 3 * D), bf16), pltpu.VMEM((D, D), bf16),
        pltpu.VMEM((3, NIT, D, FC), bf16), pltpu.VMEM((D, S), bf16),
        pltpu.VMEM((3 * HD, D), u32), pltpu.VMEM((HD, 512), u32),
        pltpu.VMEM((S // 2, D), u32), pltpu.VMEM((HD, TA), u32), pltpu.VMEM((HD, SPLIT0), u32),
        pltpu.VMEM((NG, GW // 2, S), u32), pltpu.VMEM((NG, S // 2, 128), u32),
        pltpu.VMEM((H, 16, S), u32), pltpu.VMEM((H, 32, S), f32), pltpu.VMEM((D, S), f32),
        pltpu.VMEM(((S // 128) * H, 32, 128), f32), pltpu.VMEM((NS * NTL, DH * 8, 128), f32),
        pltpu.VMEM((NS * NTL, NOFF, 128), f32), pltpu.VMEM((NS, 8, TQ), f32), pltpu.VMEM((NA * 8, TA), f32),
        pltpu.VMEM((NKB, NKG, DH * 8, 128), f32), pltpu.VMEM((NG, NOFF // 2, 128), u32),
        pltpu.VMEM((S // 2, TQ), u32), pltpu.VMEM((S, TQ), f32),
        pltpu.SemaphoreType.DMA((9,)), pltpu.SemaphoreType.DMA((1,))]

    return kernel, scratch


@jax.jit
def pallas_parallel_sum__softmax_full_mha__glu_gated_swiglu__prompt_kernel(
    A_x: jax.Array,
    A_wqkv: jax.Array,
    A_wo: jax.Array,
    B_x: jax.Array,
    B_w1: jax.Array,
    B_w3: jax.Array,
    B_w2: jax.Array,
):
    del B_x
    kernel, scratch = _build()
    anyspec = pl.BlockSpec(memory_space=pl.ANY)
    out_t = pl.pallas_call(
        kernel,
        in_specs=[anyspec] * 6,
        out_specs=anyspec,
        out_shape=jax.ShapeDtypeStruct((D, S), bf16),
        scratch_shapes=scratch,
        compiler_params=pltpu.CompilerParams(vmem_limit_bytes=100 * 1024 * 1024),
        name="fused_mha_swiglu",
    )(A_x.reshape(S, D).T, A_wqkv, A_wo, B_w1, B_w3, B_w2.T)
    return out_t.T.reshape(1, S, D)
```

```python
import functools
import math

import jax
import jax.numpy as jnp
from jax import lax
from jax.experimental import pallas as pl
from jax.experimental.pallas import tpu as pltpu

S, D, H, DH, F = 2048, 448, 16, 28, 1792
HD = D // 2
EPS = 1e-5
QSCALE = (DH ** -0.5) * math.log2(math.e)
NT = (((1,), (1,)), ((), ()))
f32, bf16, u32 = jnp.float32, jnp.bfloat16, jnp.uint32
BIG, SMALL = 2.0 ** 60, 2.0 ** -60


def _build():
    NOFF, OA = 240, 64
    TR = (13, 10, 7, 4, 1)
    FB, FPOS, FPD = (12, 4), (40, 138), 4
    WG, WU, WD = 1100, 950, 900
    BC, BSKIP, RELB = (20, 24, 12), 20, 8
    QB0, QBE = 4, 6
    TQ = TA = 512
    KC, FC, OW, OG, RS, SPLIT0 = 128, 256, 128, 2, 2, 384
    NS, LAG, AHEAD, NKB = 9, 3, 3, 8
    NQ, NC, NA, NO, NTL = S // TQ, S // KC, S // TA, S // OW, TQ // 128
    NI = NQ * H
    NIT = (NI - 1) // NS
    NKG = NOFF // 8
    NJ = NKG * NTL
    ALAST = FPOS[-1]
    assert NOFF % 16 == 0 and F // FC == NIT and sum(FB) == S // 128 and sum(BC) == 2 * DH

    def _pat(n):
        return [16 * (((c_ + 1) * (n // 16)) // 4 - (c_ * (n // 16)) // 4) for c_ in range(4)]
    OFFR = _pat(OA) * 3 + _pat(NOFF - 3 * OA)
    OFFS = [sum(OFFR[:c_]) for c_ in range(NC + 1)]
    assert OFFS[NC] == NOFF

    def kernel(xt_hbm, wqkv_hbm, wo_hbm, w1_hbm, w3_hbm, w2t_hbm, out_hbm,
               xt_ref, wqkv_ref, wo_ref, wf_ref, outb_ref,
               wt_ref, wot_ref, xn_ref, xnt_ref, kt_ref, k_ref, vt_ref, ot_ref, acc_ref,
               qf_ref, qb_ref, so_ref, mo_ref, vm_ref, kb_ref, p_ref, s_ref, sems, osem):

        def wcopy(c0, c1, k):
            return pltpu.make_async_copy(wqkv_hbm.at[:, c0:c1], wqkv_ref.at[:, c0:c1], sems.at[k])

        cp_x = [pltpu.make_async_copy(xt_hbm.at[:, c * TA:(c + 1) * TA], xt_ref.at[c], sems.at[c])
                for c in range(NA)]
        cp_wk, cp_wq, cp_wv = wcopy(384, 896, 4), wcopy(0, 384, 5), wcopy(896, 3 * D, 6)
        cp_wo = pltpu.make_async_copy(wo_hbm, wo_ref, sems.at[7])
        for cp in [cp_x[0], cp_wk, cp_wq, cp_wv] + cp_x[1:] + [cp_wo]:
            cp.start()
        acc_ref[...] = jnp.zeros((D, S), f32)
        cp_x[0].wait()
        for k, src in enumerate((w1_hbm, w3_hbm, w2t_hbm)):
            for j in range(NIT):
                pltpu.make_async_copy(src.at[:, j * FC:(j + 1) * FC], wf_ref.at[k, j], sems.at[8]).start()

        def dsl(start, size, align):
            return pl.ds(start, size) if isinstance(start, int) else pl.ds(pl.multiple_of(start, align), size)

        def first_row(n_rows, n, dtype):
            return jnp.where(lax.broadcasted_iota(jnp.int32, (n_rows, n), 0) == 0, 1.0, 0.0).astype(dtype)

        def layernorm(c):
            xt = xt_ref[c].astype(f32)
            mu = jnp.sum(xt, axis=0, keepdims=True) * (1.0 / D)
            xc = xt - mu
            var = jnp.sum(xc * xc, axis=0, keepdims=True) * (1.0 / D)
            return (xc * lax.rsqrt(var + EPS)).astype(bf16)

        def flush_k(c, rel=None):
            out = []
            if rel is not None:
                z = pltpu.bitcast(rel - rel, u32)
                z = jnp.concatenate([jnp.concatenate([z] * NTL, axis=1)] * 2, axis=0)
            for h in range(H):
                kt = kt_ref[h] if rel is None else kt_ref[h] | z
                kp = pltpu.bitcast(pltpu.bitcast(kt, bf16).T, u32)
                k_ref[h, dsl(c * (TA // 2), TA // 2, TA // 2), :] = kp
                out.append(kp)
            return out

        def proj(t0, xnt, p0, p1):
            n = xnt.shape[1]
            sl = dsl(t0, n, TA)
            yy = jnp.dot(pltpu.bitcast(wt_ref[p0 * HD:p1 * HD, :], bf16), xnt, preferred_element_type=f32)
            for part in range(p0, p1):
                y = yy[(part - p0) * D:(part - p0 + 1) * D, :]
                if part == 0:
                    pad = first_row(32 - DH, n, f32)
                    c0 = t0 if n < TA else 0
                    for h in range(H):
                        kt_ref[h, :, c0:c0 + n] = pltpu.bitcast(
                            jnp.concatenate([y[DH * h:DH * (h + 1), :], pad], axis=0).astype(bf16), u32)
                elif part == 1:
                    yq = (y * QSCALE).astype(bf16)
                    yf = yq.astype(f32)
                    for h in range(H):
                        yh = jnp.concatenate([yf[h * DH:(h + 1) * DH, :], jnp.zeros((32 - DH, n), f32)], axis=0)
                        for t in range(n // 128):
                            qf_ref[(t0 // 128 + t) * H + h] = yh[:, t * 128:(t + 1) * 128]
                else:
                    c0 = t0 % TA if n < TA else 0
                    vm_ref[dsl((t0 // TA) * 8, 8, 8), c0:c0 + n] = jnp.max(
                        jnp.abs(y).reshape(D // 8, 8, n), axis=0)
                    vpad = first_row(32 - DH, n, f32)
                    for h in range(H):
                        vt_ref[h, :, sl] = pltpu.bitcast(
                            jnp.concatenate([y[DH * h:DH * (h + 1), :], vpad], axis=0).astype(bf16), u32)
            return yy

        def head_k(kp, rel=None):
            if rel is not None:
                z = pltpu.bitcast(rel - rel, u32)[:, 0:32]
                kp = kp | jnp.concatenate([z] * (kp.shape[0] // 8), axis=0)
            return pltpu.bitcast(kp, bf16).astype(f32)

        def build_col(kf, slot, kgs, d):
            n = kf.shape[0]
            bc = jnp.broadcast_to(kf[:, d:d + 1], (n, 128))
            kb_ref[slot, kgs, d * 8:(d + 1) * 8, :] = bc.reshape(n // 8, 8, 128)
            return bc[n - 8:n, :]

        def off_keys(h, c, pat):
            return jnp.concatenate([k_ref[h, dsl(c * (TA // 2) + j * 64, r // 2, 64), :]
                                    for j, r in enumerate(pat) if r], axis=0)

        def prebuild(c, ks, pat):
            for h in range(1, 5):
                kf = head_k(jnp.concatenate([ks[h][j * 64:j * 64 + r // 2, :] for j, r in enumerate(pat) if r], axis=0))
                for d in range(DH):
                    build_col(kf, h, pl.ds(c * (OA // 8), sum(pat) // 8), d)

        def xnt_load(c0=0, c1=TA):
            return pltpu.bitcast(xnt_ref[:, c0:c1], bf16)

        xnt_ref[...] = pltpu.bitcast(layernorm(0), u32)
        cp_wk.wait()
        wt_ref[0:HD, :] = pltpu.bitcast(wqkv_ref[:, 384:896].T[64:512, :], u32)
        proj(0, xnt_load(0, SPLIT0), 0, 1)
        xn_ref[0:TA // 2, :] = pltpu.bitcast(xnt_load().T, u32)
        cp_wq.wait()
        cp_wv.wait()
        proj(SPLIT0, xnt_load(SPLIT0, TA), 0, 1)
        wt_ref[HD:2 * HD, :] = pltpu.bitcast(wqkv_ref[:, 0:512].T[0:D, :], u32)
        wt_ref[2 * HD:3 * HD, :] = pltpu.bitcast(wqkv_ref[:, 896:3 * D].T, u32)
        proj(0, xnt_load(), 1, 2)
        for cp in cp_x[1:]:
            cp.wait()

        def a_body(c, carry):
            yv = proj((c - 1) * TA, xnt_load(), 2, 3)
            xnt = layernorm(c)
            xn_ref[dsl(c * (TA // 2), TA // 2, TA // 2), :] = pltpu.bitcast(xnt.T, u32)
            proj(c * TA, xnt, 1, 2)
            ks = flush_k(c - 1, yv[D - 8:D, TA - 128:TA])
            proj(c * TA, xnt, 0, 1)
            xnt_ref[...] = pltpu.bitcast(xnt, u32)
            prebuild(c - 1, ks, OFFR[0:4])
            return carry
        lax.fori_loop(1, NA, a_body, 0)
        cp_wo.wait()

        row32 = lax.broadcasted_iota(jnp.int32, (32, TQ), 0)

        def item(i):
            return i // NQ, (i % NQ) * TQ

        def make_qm(i, cneg):
            h, q0 = item(i)
            q = jnp.concatenate([qf_ref[(q0 // 128 + t) * H + h] for t in range(NTL)], axis=1)
            if cneg is not None:
                q = jnp.where(row32 == DH, cneg, q)
            return q.astype(bf16)

        def rmax(st, m8):
            cm = jnp.max(st.reshape(st.shape[0] // 8, 8, TQ), axis=0)
            return cm if m8 is None else jnp.maximum(m8, cm)

        def pv_unit(i, u, acc):
            p = pltpu.bitcast(p_ref[u * KC // 2:(u + 1) * KC // 2, :], bf16)
            vt = pltpu.bitcast(vt_ref[item(i)[0], :, u * KC:(u + 1) * KC], bf16)
            pv = jnp.dot(vt, p, preferred_element_type=f32)
            return pv if acc is None else acc + pv

        def finish(i, acc, chk):
            h, q0 = item(i)
            ot_ref[h, :, dsl(q0, TQ, TQ)] = acc
            return jnp.maximum(chk[0], acc[24:32, :]), jnp.minimum(chk[1], acc[24:32, :])

        def build_qb(i, k, n, z):
            h, q0 = item(i)
            t, gq = divmod(n, 4)
            nr = min(8, DH - gq * 8)
            q = qf_ref[(q0 // 128 + t) * H + h, gq * 8:(gq + 1) * 8, :] + z
            qb_ref[k * NTL + t, gq * 64:gq * 64 + nr * 8, :] = jnp.concatenate(
                [jnp.broadcast_to(q[d:d + 1, :], (8, 128)) for d in range(nr)], axis=0)

        def stage(i, s, acc, chk, hook, first=False, extra=None):
            h = item(i)[0]
            cneg = -(jnp.max(mo_ref[s], axis=0, keepdims=True).astype(bf16).astype(f32))
            qm = make_qm(i, cneg)
            for c in range(NC):
                if c >= LAG:
                    acc = pv_unit(i, c - LAG, acc)
                elif not first:
                    acc = pv_unit(i - 1, NC - LAG + c, acc)
                    if c == LAG - 1:
                        chk = finish(i - 1, acc, chk)
                        acc = None
                r0, r1 = c * KC + OFFR[c], (c + 1) * KC
                st = jnp.dot(pltpu.bitcast(k_ref[h, r0 // 2:r1 // 2, :], bf16), qm, preferred_element_type=f32)
                st = hook(st, s * NC + c)
                if OFFR[c]:
                    so = jnp.concatenate([so_ref[s * NTL + t, OFFS[c]:OFFS[c + 1], :] for t in range(NTL)], axis=1)
                    st = jnp.concatenate([so + cneg, st], axis=0)
                p_ref[c * KC // 2:(c + 1) * KC // 2, :] = pltpu.bitcast(jnp.exp2(st).astype(bf16), u32)
                if extra is not None:
                    extra(s * NC + c)
            return acc, chk

        ks = flush_k(NA - 1)
        proj((NA - 1) * TA, xnt_load(0, 128), 2, 3)
        for i_ in range(AHEAD + 1):
            val = jnp.dot(pltpu.bitcast(off_keys(0, 0, OFFR), bf16), make_qm(i_, None), preferred_element_type=f32)
            for t in range(NTL):
                so_ref[((i_ - 1) % NS) * NTL + t] = val[:, t * 128:(t + 1) * 128]
            mo_ref[(i_ - 1) % NS] = rmax(val, None)
        proj((NA - 1) * TA + 128, xnt_load(128, TA), 2, 3)
        zpad4 = jnp.zeros((32 - DH, D), f32)
        wof = wo_ref[...].astype(f32)
        wop = jnp.concatenate(
            [blk for h in range(H) for blk in (wof[h * DH:(h + 1) * DH, :], zpad4)], axis=0)
        wot_ref[...] = pltpu.bitcast(wop.astype(bf16).T, u32)
        prebuild(NA - 1, ks, OFFR[12:16])

        def hook0(st, n):
            for k in range(NS):
                v = st[(k + 2) * 8:(k + 3) * 8, 0:128]
                build_qb(k + AHEAD + 1, k, n % NC, v - v)
            return st
        one = jnp.ones((8, TQ), f32)
        carry0 = stage(0, NS - 1, None, (one, one), hook0, first=True)

        pltpu.make_async_copy(wf_ref, wf_ref, sems.at[8]).wait()

        def split_tie(y, pos, fn):
            R, C = y.shape[0] // 8, y.shape[1] // 128
            newv = {(r, c): fn(y[r * 8:(r + 1) * 8, c * 128:(c + 1) * 128]) for (r, c) in pos}
            cols = []
            for c in range(C):
                pieces, lo = [], 0
                for r in sorted(r for (r, c_) in newv if c_ == c):
                    if r > lo:
                        pieces.append(y[lo * 8:r * 8, c * 128:(c + 1) * 128])
                    pieces.append(newv[(r, c)])
                    lo = r + 1
                if lo < R:
                    pieces.append(y[lo * 8:R * 8, c * 128:(c + 1) * 128])
                cols.append(pieces[0] if len(pieces) == 1 else jnp.concatenate(pieces, axis=0))
            return jnp.concatenate(cols, axis=1)

        def spread(y, n, skip, pair):
            R, C = y.shape[0] // 8, y.shape[1] // 128
            lo = (R * C * skip) // 100
            idx = [lo + ((k + 1) * (R * C - lo)) // n - 1 for k in range(n)]
            if pair:
                return [((i_ % (2 * R)) // 2, 2 * (i_ // (2 * R)) + i_ % 2) for i_ in idx]
            return [(i_ % R, i_ // R) for i_ in idx]

        def att_body(t, carry):
            heads = [item(jnp.minimum(t * NS + k + AHEAD + 1, NI - 1))[0] for k in range(NS)]
            n_ffn = NS * NJ - (ALAST + 1) * len(TR)
            total = sum(FB[:-1]) * (WG + WU + WD)
            st_ = {"time": 0, "fdone": 0, "done": 0, "step": 0, "nb": 0}
            mx = [None] * NTL
            hstate = {}

            def qb_next(k, n, z):
                build_qb(jnp.minimum((t + 1) * NS + k + AHEAD + 1, NI - 1), k, n, z)

            def chain_tie(v):
                k, n_in = divmod(st_["done"], NJ)
                kg, tt = divmod(n_in, NTL)
                slot = (k + AHEAD) % NS
                assert (k + AHEAD - NS + 1) * NC <= st_["step"] < (k + AHEAD) * NC
                st_["done"] += 1
                pr = (kb_ref[heads[k] % NKB, kg] * qb_ref[k * NTL + tt]).reshape(DH // 2, 16, 128)
                s2 = jnp.sum(pr, axis=0)
                res = s2[0:8] + s2[8:16]
                so_ref[slot * NTL + tt, kg * 8:(kg + 1) * 8, :] = res
                mx[tt] = res if kg == 0 else jnp.maximum(mx[tt], res)
                if kg == NKG - 1:
                    mo_ref[slot, :, tt * 128:(tt + 1) * 128] = mx[tt]
                z = mx[tt] - mx[tt]
                nq = n_in - QB0
                if k > 0 and nq >= 0 and nq % QBE == 0 and nq // QBE < 16:
                    qb_next(k - 1, nq // QBE, z)
                return v + z

            def build_tie(v):
                k_, d = divmod(st_["nb"], DH)
                st_["nb"] += 1
                hb = 5 + 2 * t + k_
                if d == 0:
                    hc = jnp.minimum(hb, H - 1)
                    st_["kf"] = head_k(off_keys(hc, 0, OFFR), st_["rel"])
                res = build_col(st_["kf"], hb % NKB, slice(None), d)
                z = res - res
                v = v + z
                if st_["nb"] % 3 == 0 and st_["nb"] // 3 <= 16:
                    qb_next(NS - 1, st_["nb"] // 3 - 1, z)
                if d == DH - RELB:
                    st_["rel"] = v
                return v

            def tie(y, b, w, kind):
                pair = kind == 2
                if b == len(FB) - 1:
                    return split_tie(y, spread(y, BC[kind], BSKIP if kind == 0 else 0, pair), build_tie)
                st_["time"] += w * FB[b]
                n = (n_ffn * st_["time"]) // total - st_["fdone"]
                st_["fdone"] += n
                return split_tie(y, spread(y, n, 0, pair), chain_tie)

            def hook(st, n):
                st_["step"] = n
                if n == ALAST:
                    st_["rel"] = st[0:8, 0:128]
                if n > ALAST:
                    return st
                return split_tie(st, [(st.shape[0] // 8 - r, k % NTL) for k, r in enumerate(TR)], chain_tie)

            def ffn_up(b):
                t0, t1 = sum(FB[:b]) * 128, sum(FB[:b + 1]) * 128
                xq = pltpu.bitcast(xn_ref[t0 // 2:t1 // 2, :], bf16)
                gt = tie(jnp.dot(xq, wf_ref[0, t], preferred_element_type=f32), b, WG, 0)
                up = tie(jnp.dot(xq, wf_ref[1, t], preferred_element_type=f32), b, WU, 1)
                gh = 0.5 * gt
                hstate[b] = ((gh * up) * (jnp.tanh(gh) + 1.0)).astype(bf16)

            def ffn_down(b):
                t0, t1 = sum(FB[:b]) * 128, sum(FB[:b + 1]) * 128
                dn = lax.dot_general(wf_ref[2, t], hstate.pop(b), NT, preferred_element_type=f32)
                acc_ref[:, t0:t1] += tie(dn, b, WD, 2)

            sched = {}
            for b in range(len(FB)):
                sched[FPOS[b]] = functools.partial(ffn_up, b)
                sched[FPOS[b] + FPD] = functools.partial(ffn_down, b)

            def extra(n):
                if n in sched:
                    sched[n]()

            for s in range(NS):
                carry = stage(t * NS + s + 1, s, *carry, hook, extra=extra)
            assert st_["done"] == NS * NJ and st_["nb"] == 2 * DH
            return carry

        acc, chk = lax.fori_loop(0, NIT, att_body, carry0)

        RH, PB = D // RS, TA // OW
        state = {"n": 0, "lo": 0}

        def normalized(sl):
            a = ot_ref[:, :, sl]
            l = a[:, DH:DH + 1, :]
            r0 = pl.reciprocal(l, approx=True)
            r0 = r0 * (2.0 - l * r0)
            return (a * r0).reshape(H * 32, OW).astype(bf16)

        def next_piece():
            b, r = divmod(state["n"], RS)
            sl = slice(b * OW, (b + 1) * OW)
            rs = slice(r * RH, (r + 1) * RH)
            if r == 0:
                state["o"] = normalized(sl)
            wo_t = pltpu.bitcast(wot_ref[r * RH // 2:(r + 1) * RH // 2, :], bf16)
            x = xt_ref[b // PB, rs, (b % PB) * OW:(b % PB + 1) * OW].astype(f32)
            o = (x + acc_ref[rs, sl]) + jnp.dot(wo_t, state["o"], preferred_element_type=f32)
            outb_ref[rs, sl] = o.astype(bf16)
            state["n"] += 1
            if r == RS - 1 and ((b + 1) % OG == 0 or b + 1 >= NO - 1):
                c0, c1 = state["lo"] * OW, (b + 1) * OW
                pltpu.make_async_copy(outb_ref.at[:, c0:c1], out_hbm.at[:, c0:c1], osem.at[0]).start()
                state["lo"] = b + 1

        for c in range(LAG):
            acc = pv_unit(NI - 1, NC - LAG + c, acc)
            next_piece()
        chk = finish(NI - 1, acc, chk)
        while state["n"] < NO * RS:
            next_piece()
        lhi, llo = chk[0][DH - 24:DH - 23, :], chk[1][DH - 24:DH - 23, :]
        ok = (lhi < BIG) & (llo > SMALL) & (jnp.max(vm_ref[...], axis=0, keepdims=True) < BIG)
        bad = jnp.max(jnp.where(ok, 0.0, 1.0))
        pltpu.make_async_copy(outb_ref, out_hbm, osem.at[0]).wait()

        @pl.when(bad > 0.0)
        def _():
            def fb_item(i, carry):
                h, q0 = item(i)
                qm = make_qm(i, None)

                def qk(c, m8):
                    kk = pltpu.bitcast(k_ref[h, dsl(c * (KC // 2), KC // 2, KC // 2), :], bf16)
                    st = jnp.dot(kk, qm, preferred_element_type=f32)
                    s_ref[dsl(c * KC, KC, KC), :] = st
                    return rmax(st, m8)
                m8 = lax.fori_loop(0, NC, qk, jnp.full((8, TQ), -jnp.inf, f32))
                m = jnp.max(m8, axis=0, keepdims=True)

                def pv(c, a):
                    p = jnp.exp2(s_ref[dsl(c * KC, KC, KC), :] - m).astype(bf16)
                    vt = pltpu.bitcast(vt_ref[h, :, dsl(c * KC, KC, KC)], bf16)
                    return a + jnp.dot(vt, p, preferred_element_type=f32)
                ot_ref[h, :, dsl(q0, TQ, TQ)] = lax.fori_loop(0, NC, pv, jnp.zeros((32, TQ), f32))
                return carry
            lax.fori_loop(0, NI, fb_item, 0)

            def fb_out(b, carry):
                sl = dsl(b * OW, OW, OW)
                x = xt_ref[b // PB, :, dsl((b % PB) * OW, OW, OW)].astype(f32)
                o = (x + acc_ref[:, sl]) + jnp.dot(
                    pltpu.bitcast(wot_ref[...], bf16), normalized(sl), preferred_element_type=f32)
                outb_ref[:, sl] = o.astype(bf16)
                return carry
            lax.fori_loop(0, NO, fb_out, 0)
            cp = pltpu.make_async_copy(outb_ref, out_hbm, osem.at[0])
            cp.start()
            cp.wait()

    scratch = [
        pltpu.VMEM((NA, D, TA), bf16), pltpu.VMEM((D, 3 * D), bf16), pltpu.VMEM((D, D), bf16),
        pltpu.VMEM((3, NIT, D, FC), bf16), pltpu.VMEM((D, S), bf16),
        pltpu.VMEM((3 * HD, D), u32), pltpu.VMEM((HD, 512), u32),
        pltpu.VMEM((S // 2, D), u32), pltpu.VMEM((HD, TA), u32), pltpu.VMEM((H, 16, TA), u32),
        pltpu.VMEM((H, S // 2, 32), u32),
        pltpu.VMEM((H, 16, S), u32), pltpu.VMEM((H, 32, S), f32), pltpu.VMEM((D, S), f32),
        pltpu.VMEM(((S // 128) * H, 32, 128), f32), pltpu.VMEM((NS * NTL, DH * 8, 128), f32),
        pltpu.VMEM((NS * NTL, NOFF, 128), f32), pltpu.VMEM((NS, 8, TQ), f32), pltpu.VMEM((NA * 8, TA), f32),
        pltpu.VMEM((NKB, NKG, DH * 8, 128), f32),
        pltpu.VMEM((S // 2, TQ), u32), pltpu.VMEM((S, TQ), f32),
        pltpu.SemaphoreType.DMA((9,)), pltpu.SemaphoreType.DMA((1,))]

    return kernel, scratch


@jax.jit
def pallas_parallel_sum__softmax_full_mha__glu_gated_swiglu__prompt_kernel(
    A_x: jax.Array,
    A_wqkv: jax.Array,
    A_wo: jax.Array,
    B_x: jax.Array,
    B_w1: jax.Array,
    B_w3: jax.Array,
    B_w2: jax.Array,
):
    del B_x
    kernel, scratch = _build()
    anyspec = pl.BlockSpec(memory_space=pl.ANY)
    out_t = pl.pallas_call(
        kernel,
        in_specs=[anyspec] * 6,
        out_specs=anyspec,
        out_shape=jax.ShapeDtypeStruct((D, S), bf16),
        scratch_shapes=scratch,
        compiler_params=pltpu.CompilerParams(vmem_limit_bytes=100 * 1024 * 1024),
        name="fused_mha_swiglu",
    )(A_x.reshape(S, D).T, A_wqkv, A_wo, B_w1, B_w3, B_w2.T)
    return out_t.T.reshape(1, S, D)
```
